```python
import os as _os
_os.environ.setdefault('JAX_PLATFORMS', 'cpu')
import jax
import jax.numpy as jnp

def _softmax(x, axis=-1):
    return jax.nn.softmax(x, axis=axis)

def _gelu(x):
    return jax.nn.gelu(x, approximate=True)

def _silu(x):
    return jax.nn.silu(x)

def _sigmoid(x):
    return jax.nn.sigmoid(x)

def _layernorm(x, axis=-1, eps=1e-05):
    m = jnp.mean(x, axis=axis, keepdims=True)
    v = jnp.var(x, axis=axis, keepdims=True)
    return (x - m) / jnp.sqrt(v + eps)

def _scatter_add(tgt, idx, src, axis=0):
    return tgt.at[idx].add(src)

def _segment_sum(src, seg, n):
    return jax.ops.segment_sum(src, seg, n)

class _Rng:

    def __init__(self, key):
        self._k = key

    def _next(self):
        self._k, sub = jax.random.split(self._k)
        return sub

    def normal(self, shape):
        return jax.random.normal(self._next(), shape, dtype=jnp.bfloat16)

    def randint(self, lo, hi, shape):
        return jax.random.randint(self._next(), shape, lo, hi, dtype=jnp.int32)

    def uniform(self, shape, lo=0.0, hi=1.0):
        return jax.random.uniform(self._next(), shape, jnp.bfloat16, lo, hi)

    def permutation(self, n):
        return jax.random.permutation(self._next(), n)
kernel_name = 'parallel_sum__memory_aug_recurrent_mem_tr__dense_activation_gelu__prompt'

def setup_inputs():
    _rng = _Rng(jax.random.key(int.from_bytes(__import__("os").urandom(4), "little")))
    _w = lambda a: (lambda t: t.astype(jnp.bfloat16) if jnp.issubdtype(t.dtype, jnp.floating) else t)(jnp.asarray(a))

    def _A_setup():
        B, S, Dm = (1, 2048, 1024)
        H, Dh = (32, 128)
        M, seg = (8, 32)
        seg = min(seg, S)
        S = S // seg * seg
        return {'x': _w((lambda *s: _rng.normal(s) * 0.05)(B, S, Dm)), 'mem0': _w((lambda *s: _rng.normal(s) * 0.2)(B, M, Dm)), 'Wq': _w((lambda *s: _rng.normal(s) * 0.8)(Dm, H, Dh) * Dm ** (-0.5)), 'Wk': _w((lambda *s: _rng.normal(s) * 0.8)(Dm, H, Dh) * Dm ** (-0.5)), 'Wv': _w((lambda *s: _rng.normal(s) * 0.2)(Dm, H, Dh) * Dm ** (-0.5)), 'Wo': _w((lambda *s: _rng.normal(s) * 0.2)(H, Dh, Dm) * (H * Dh) ** (-0.5)), 'seg_len': seg}
    _A_in = _A_setup()

    def _B_setup():
        B, S, D, F = (1, 2048, 1024, 3584)
        return {'x': _w((lambda *s: _rng.normal(s) * 0.05)(B, S, D)), 'w1': _w((lambda *s: _rng.normal(s) * 0.1)(D, F) * D ** (-0.5)), 'b1': _w((lambda *s: _rng.normal(s) * 0.1)(F) * 0.01), 'w2': _w((lambda *s: _rng.normal(s) * 0.1)(F, D) * F ** (-0.5)), 'b2': _w((lambda *s: _rng.normal(s) * 0.05)(D) * 0.01)}
    _B_in = _B_setup()
    return {'A_x': _A_in['x'], 'A_mem0': _A_in['mem0'], 'A_Wq': _A_in['Wq'], 'A_Wk': _A_in['Wk'], 'A_Wv': _A_in['Wv'], 'A_Wo': _A_in['Wo'], 'A_seg_len': _A_in['seg_len'], 'B_x': _B_in['x'], 'B_w1': _B_in['w1'], 'B_b1': _B_in['b1'], 'B_w2': _B_in['w2'], 'B_b2': _B_in['b2']}

def reference(A_x, A_mem0, A_Wq, A_Wk, A_Wv, A_Wo, A_seg_len, B_x, B_w1, B_b1, B_w2, B_b2):

    def _A_ref(x, mem0, Wq, Wk, Wv, Wo, seg_len):
        B, S, Dm = x.shape
        H, Dh = (Wq.shape[1], Wq.shape[2])
        M = mem0.shape[1]
        scale = Dh ** (-0.5)
        n_seg = S // seg_len
        L = M + seg_len
        idx = jnp.arange(L)
        mask = (idx[:, None] < M) | (idx[:, None] >= idx[None, :])
        mem = mem0
        outs = []
        for s in range(n_seg):
            xs = x[:, s * seg_len:(s + 1) * seg_len, :].copy()
            h = jnp.concatenate([mem, xs], axis=1)
            q = jnp.einsum('btd,dhe->bhte', h, Wq)
            k = jnp.einsum('btd,dhe->bhte', h, Wk)
            v = jnp.einsum('btd,dhe->bhte', h, Wv)
            scores = jnp.einsum('bhqe,bhke->bhqk', q, k) * scale
            scores = jnp.where(mask[None, None], scores, -1000000000.0)
            p = _softmax(scores, axis=-1)
            o = jnp.einsum('bhqk,bhke->bhqe', p, v)
            o = jnp.einsum('bhte,hed->btd', o, Wo)
            mem = o[:, :M, :].copy()
            outs.append(o[:, M:, :])
        return jnp.concatenate(outs, axis=1)

    def _B_ref(x, w1, b1, w2, b2):
        h = jnp.einsum('bsd,df->bsf', x, w1) + b1
        h = _gelu(h)
        return jnp.einsum('bsf,fd->bsd', h, w2) + b2
    x = A_x
    xn = _layernorm(x, axis=-1)
    return x + _A_ref(xn, A_mem0, A_Wq, A_Wk, A_Wv, A_Wo, A_seg_len) + _B_ref(xn, B_w1, B_b1, B_w2, B_b2)
```

```python
import functools
import jax, jax.numpy as jnp, numpy as np
from jax import lax
from jax.experimental import pallas as pl
from jax.experimental.pallas import tpu as pltpu

BF = jnp.bfloat16
F32 = jnp.float32
U32 = jnp.uint32

def _bc(x):
    return pltpu.bitcast(x, BF)

def _pk(x):
    return pltpu.bitcast(x.astype(BF), U32)

def _mm(a, b):
    return jnp.dot(a, b, preferred_element_type=F32)

def _gelu(x):
    c = 0.7978845608028654
    return 0.5 * x * (1.0 + jnp.tanh(c * (x + 0.044715 * (x * x * x))))

def _ds(start, size, mult):
    return pl.ds(pl.multiple_of(start, mult), size)

def make_kernel(S, Dm, H, Dh, M, seg, F, opts):
    KT = Dm // 128
    FT = F // 128
    HD = H * Dh
    scale = float(Dh) ** -0.5
    L = M + seg
    NIT = S // 64
    o_f1 = opts.get('f1', (6, 6))

    def kernel(mem0_ref, b1_ref, b2_ref, x_h, wq_h, wk_h, wv_h, wo_h, w1_h, w2_h,
               o_ref,
               wqkv, wo, w1, w2, stg, XR, XN, XBlo, XBhi, Hp, FFO, sems,
               mem_s, carry, oleft, OA, OB, Hs, FF, B1f, B2f):
        it = pl.program_id(0)

        def layernorm_rows(r0, nrows):
            x = XR[_ds(r0, nrows, 64), :].astype(F32)
            mu = jnp.mean(x, axis=-1, keepdims=True)
            xc = x - mu
            var = jnp.mean(xc * xc, axis=-1, keepdims=True)
            xn = xc * lax.rsqrt(var + 1e-5)
            XN[_ds(r0, nrows, 64), :] = xn
            nb = nrows // 64
            lo = jnp.concatenate([xn[64 * i:64 * i + 32] for i in range(nb)], axis=0)
            hi = jnp.concatenate([xn[64 * i + 32:64 * i + 64] for i in range(nb)], axis=0)
            XBlo[_ds(r0 // 4, nrows // 4, 16), :] = _pk(lo)
            XBhi[_ds(r0 // 4, nrows // 4, 16), :] = _pk(hi)

        def relayout_piece(p):
            s32 = stg.bitcast(U32)
            blk = s32.at[_ds(p * 256, 256, 256)]
            m = p // 64
            r0 = (p % 64) * 8
            for hp in range(16):
                A = blk[pl.ds(hp, 8, stride=32), :]
                B = blk[pl.ds(16 + hp, 8, stride=32), :]
                lo = (A & 0xFFFF) | (B << 16)
                hi = (A >> 16) | (B & np.uint32(0xFFFF0000))
                wqkv[m * H + 2 * hp, _ds(r0, 8, 8), :] = lo
                wqkv[m * H + 2 * hp + 1, _ds(r0, 8, 8), :] = hi

        @pl.when(it == 0)
        def _prologue():
            mem_s[...] = mem0_ref[...].astype(F32)
            B1f[...] = b1_ref[...].astype(F32)
            B2f[...] = b2_ref[...].astype(F32)
            sem_i = [0]
            def nsem():
                s = sems.at[sem_i[0]]; sem_i[0] += 1
                return s
            cx = [pltpu.make_async_copy(x_h.at[pl.ds(i * 1024, 1024)], XR.at[pl.ds(i * 1024, 1024)], nsem()) for i in range(2)]
            w1_32 = w1_h.bitcast(U32); w2_32 = w2_h.bitcast(U32); wo_32 = wo_h.bitcast(U32)
            S_W1 = sem_i[0]
            cw1 = [pltpu.make_async_copy(w1_32.at[:, pl.ds(j * 128, 128)], w1.at[j], nsem()) for j in range(FT)]
            S_W2 = sem_i[0]
            cw2 = [pltpu.make_async_copy(w2_32.at[:, pl.ds(j * 128, 128)], w2.at[j], nsem()) for j in range(KT)]
            S_QKV = sem_i[0]
            cq = []
            for m, wh in enumerate((wq_h, wk_h, wv_h)):
                for c in range(16):
                    cq.append(pltpu.make_async_copy(wh.at[pl.ds(c * 2048, 2048)],
                                                    stg.at[pl.ds((m * 16 + c) * 2048, 2048)], nsem()))
            cwo = [pltpu.make_async_copy(wo_32.at[:, pl.ds(j * 128, 128)], wo.at[j], nsem()) for j in range(KT)]
            cx[0].start()
            for c in cw1: c.start()
            cx[1].start()
            for c in cw2: c.start()
            for c in cq: c.start()
            for c in cwo: c.start()

            cx[0].wait()
            def ln_body(i, _):
                layernorm_rows(i * 128, 128)
                return 0
            lax.fori_loop(0, 8, ln_body, 0)

            def p1(b, side):
                def body(q, _):
                    g = q // 2
                    half = q % 2
                    @pl.when((half == 0) & (b == 0))
                    def _():
                        for t in range(7):
                            pltpu.make_async_copy(w1.at[0], w1.at[0], sems.at[S_W1 + g * 7 + t]).wait()
                    side(q)
                    lhs = _bc(XBlo[_ds(b * 256 + half * 128, 128, 128), :])
                    for t in range(7):
                        j = g * 7 + t
                        hh = _mm(lhs, _bc(w1[j])) + B1f[pl.ds(j, 1), :]
                        Hp[half, :, _ds(j * 128, 128, 128)] = _pk(_gelu(hh))
                    return 0
                lax.fori_loop(0, 8, body, 0)

            def p2(b, side):
                def body(q, _):
                    g = q // 2
                    half = q % 2
                    @pl.when((half == 0) & (b == 0))
                    def _():
                        for t in range(2):
                            pltpu.make_async_copy(w2.at[0], w2.at[0], sems.at[S_W2 + g * 2 + t]).wait()
                    side(q)
                    lhs = _bc(Hp[half])
                    for t in range(2):
                        n = g * 2 + t
                        ff = _mm(lhs, _bc(w2[n])) + B2f[pl.ds(n, 1), :]
                        FFO[_ds(b * 512 + half * 256, 256, 256), _ds(n * 128, 128, 128)] = ff
                    return 0
                lax.fori_loop(0, 8, body, 0)

            def side_none(q):
                pass

            def side_ln(q):
                layernorm_rows(1024 + q * 128, 128)

            def side_rl(base):
                def f(q):
                    r = base + q
                    for t in range(3):
                        pltpu.make_async_copy(stg.at[pl.ds(0, 2048)], stg.at[pl.ds(0, 2048)],
                                              sems.at[S_QKV + r * 3 + t]).wait()
                    for t in range(12):
                        relayout_piece(r * 12 + t)
                return f

            p1(0, side_none)
            cx[1].wait()
            p2(0, side_ln)
            p1(1, side_rl(0))
            p2(1, side_rl(8))
            for c in cwo: c.wait()

        r64 = it * 64
        xnA = XN[_ds(r64, 40, 64), :]
        xnB = XN[_ds(r64 + 40, 24, 8), :]
        xh = _bc(XBhi[_ds(it * 16, 16, 16), :])

        row = lax.broadcasted_iota(jnp.int32, (48, 48), 0)
        col = lax.broadcasted_iota(jnp.int32, (48, 48), 1)
        mask = ((row < M) | (row >= col)) & (col < L)
        c2 = scale * 1.4426950408889634

        def qk(q, k):
            return lax.dot_general(q, k, (((1,), (1,)), ((), ())), preferred_element_type=F32)

        def soft(s):
            s = jnp.where(mask, s * c2, -1e30)
            m = jnp.max(s, axis=-1, keepdims=True)
            e = jnp.exp2(s - m)
            l = jnp.sum(e, axis=-1, keepdims=True)
            r = pl.reciprocal(l, approx=True)
            r = r * (2.0 - l * r)
            return e.astype(BF), r

        def ffn1(j):
            hh = _mm(xh, _bc(w1[j])) + B1f[j:j + 1, :]
            Hs[:, j * 128:(j + 1) * 128] = _pk(_gelu(hh))

        def ffn2(j):
            FF[:, j * 128:(j + 1) * 128] = _mm(_bc(Hs[...]), _bc(w2[j])) + B2f[j:j + 1, :]

        def run_pass(lhs, asm, emit, mid, fill):
            st = {}
            for t in range(H + 2):
                if t < H:
                    q = asm(_mm(lhs, _bc(wqkv[t])), t).astype(BF)
                    k = asm(_mm(lhs, _bc(wqkv[H + t])), H + t).astype(BF)
                else:
                    for f in fill[t - H]:
                        f()
                if 1 <= t <= H:
                    qq, kk = st[t - 1]['q'], st[t - 1]['k']
                    st[t - 1]['e'], st[t - 1]['r'] = soft(qk(qq, kk))
                if t < H:
                    v = asm(_mm(lhs, _bc(wqkv[2 * H + t])), 2 * H + t).astype(BF)
                    st[t] = dict(q=q, k=k, v=v)
                    for f in mid.get(t, []):
                        f()
                if 2 <= t <= H + 1:
                    d = st.pop(t - 2)
                    o = _mm(d['e'], d['v']) * d['r']
                    emit(t - 2, o)

        mem = mem_s[...]
        lhsA = jnp.concatenate([mem, xnA], axis=0).astype(BF)

        def asmA(r, idx):
            carry[:, idx * 128:(idx + 1) * 128] = r[40:48]
            return r

        def emitA(h, o):
            OA[:, h * 128:(h + 1) * 128] = _pk(jnp.concatenate([o[0:8], o[16:40]], axis=0))
            oleft[:, h * 128:(h + 1) * 128] = o[8:16]

        f1 = [functools.partial(ffn1, j) for j in range(FT)]
        n1, n2 = o_f1
        nmid = FT - n1 - n2
        mid = {}
        for i in range(nmid):
            mid.setdefault((i * H) // nmid, []).append(f1[i])
        a0 = nmid
        run_pass(lhsA, asmA, emitA, mid, [f1[a0:a0 + n1 // 2], f1[a0 + n1 // 2:a0 + n1]])
        outA = []
        for j in range(KT):
            outA.append(_mm(_bc(OA[...]), _bc(wo[j])))
        memB = jnp.concatenate([a[0:8] for a in outA], axis=1)
        for f in f1[a0 + n1:]:
            f()

        lhsB = jnp.concatenate([memB, xnB], axis=0).astype(BF)
        z8 = jnp.zeros((8, 128), F32)

        def asmB(r, idx):
            return jnp.concatenate([r[0:8], carry[:, idx * 128:(idx + 1) * 128], r[8:32], z8], axis=0)

        def emitB(h, o):
            OB[:, h * 128:(h + 1) * 128] = _pk(jnp.concatenate(
                [o[0:8], oleft[:, h * 128:(h + 1) * 128], o[8:40]], axis=0))

        run_pass(lhsB, asmB, emitB, {}, [[functools.partial(ffn2, 0)], [functools.partial(ffn2, 1)]])
        for j in range(KT):
            ob = _mm(_bc(OB[...]), _bc(wo[j]))
            if j + 2 < KT:
                ffn2(j + 2)
            mem_s[:, j * 128:(j + 1) * 128] = ob[0:8]
            a = outA[j]
            att = jnp.concatenate([ob[8:16], a[8:32], ob[16:48]], axis=0)
            ff = jnp.concatenate([FFO[_ds(it * 32, 32, 32), j * 128:(j + 1) * 128],
                                  FF[:, j * 128:(j + 1) * 128]], axis=0)
            xr = XR[_ds(r64, 64, 64), j * 128:(j + 1) * 128].astype(F32)
            res = xr + att + ff
            o_ref[:, j * 128:(j + 1) * 128] = res.astype(BF)

    scratch = [
        pltpu.VMEM((3 * H, Dm // 2, 128), U32),
        pltpu.VMEM((KT, HD // 2, 128), U32),
        pltpu.VMEM((FT, Dm // 2, 128), U32),
        pltpu.VMEM((KT, F // 2, 128), U32),
        pltpu.VMEM((3 * Dm * H, 128), BF),
        pltpu.VMEM((S, Dm), BF),
        pltpu.VMEM((S, Dm), F32),
        pltpu.VMEM((S // 4, Dm), U32),
        pltpu.VMEM((S // 4, Dm), U32),
        pltpu.VMEM((2, 128, F), U32),
        pltpu.VMEM((S // 2, Dm), F32),
        pltpu.SemaphoreType.DMA((2 + FT + KT + 48 + KT,)),
        pltpu.VMEM((M, Dm), F32),
        pltpu.VMEM((8, 3 * HD), F32),
        pltpu.VMEM((8, HD), F32),
        pltpu.VMEM((16, HD), U32),
        pltpu.VMEM((24, HD), U32),
        pltpu.VMEM((16, F), U32),
        pltpu.VMEM((32, Dm), F32),
        pltpu.VMEM((FT, 128), F32),
        pltpu.VMEM((KT, 128), F32),
    ]
    return kernel, scratch


@functools.partial(jax.jit, static_argnames=("A_seg_len",))
def pallas_parallel_sum__memory_aug_recurrent_mem_tr__dense_activation_gelu__prompt_kernel(A_x, A_mem0, A_Wq, A_Wk, A_Wv, A_Wo, A_seg_len, B_x, B_w1, B_b1, B_w2, B_b2):
    Bn, S, Dm = A_x.shape
    _, H, Dh = A_Wq.shape
    M = A_mem0.shape[1]
    F = B_w1.shape[1]
    seg = A_seg_len
    kernel, scratch = make_kernel(S, Dm, H, Dh, M, seg, F, {})
    TB = 2 * seg
    any_spec = pl.BlockSpec(memory_space=pl.ANY)
    out = pl.pallas_call(
        kernel,
        grid=(S // TB,),
        in_specs=[
            pl.BlockSpec((M, Dm), lambda i: (0, 0)),
            pl.BlockSpec((F // 128, 128), lambda i: (0, 0)),
            pl.BlockSpec((Dm // 128, 128), lambda i: (0, 0)),
            any_spec, any_spec, any_spec, any_spec, any_spec, any_spec, any_spec,
        ],
        out_specs=pl.BlockSpec((TB, Dm), lambda i: (i, 0)),
        out_shape=jax.ShapeDtypeStruct((S, Dm), A_x.dtype),
        scratch_shapes=scratch,
        compiler_params=pltpu.CompilerParams(
            dimension_semantics=("arbitrary",),
            vmem_limit_bytes=120 * 1024 * 1024),
    )(A_mem0.reshape(M, Dm), B_b1.reshape(F // 128, 128), B_b2.reshape(Dm // 128, 128),
      A_x.reshape(S, Dm),
      A_Wq.reshape(Dm * H, Dh), A_Wk.reshape(Dm * H, Dh), A_Wv.reshape(Dm * H, Dh),
      A_Wo.reshape(H * Dh, Dm), B_w1, B_w2)
    return out.reshape(Bn, S, Dm)
```

```python
import functools
import jax, jax.numpy as jnp, numpy as np
from jax import lax
from jax.experimental import pallas as pl
from jax.experimental.pallas import tpu as pltpu

BF = jnp.bfloat16
F32 = jnp.float32
U32 = jnp.uint32

def _bc(x):
    return pltpu.bitcast(x, BF)

def _pk(x):
    return pltpu.bitcast(x.astype(BF), U32)

def _mm(a, b):
    return jnp.dot(a, b, preferred_element_type=F32)

def _gelu(x):
    c = 0.7978845608028654
    return 0.5 * x * (1.0 + jnp.tanh(c * (x + 0.044715 * (x * x * x))))

def _ds(start, size, mult):
    if isinstance(start, int):
        return pl.ds(start, size)
    return pl.ds(pl.multiple_of(start, mult), size)

def make_kernel(S, Dm, H, Dh, M, seg, F, opts):
    KT = Dm // 128
    FT = F // 128
    HD = H * Dh
    scale = float(Dh) ** -0.5
    L = M + seg
    NIT = S // 64
    TR = 72
    unr = opts.get('unr', 1)
    rl = opts.get('rl', [8, 20, 20])
    assert sum(rl) * 4 == 192
    full = opts.get('full', False)
    MB1 = opts.get('mb1', 256)
    MB2 = opts.get('mb2', 256)
    o_f1 = tuple(opts.get('f1', (3, 6, 6)))

    def kernel(mem0_ref, b1_ref, b2_ref, x_h, wq_h, wk_h, wv_h, wo_h, w1_h, w2_h,
               o_ref,
               wqkv, wo, w1, w2, stg, XR, XN, XBlo, XBhi, Hp, FFO, sems,
               mem_s, carry, oleft, OA, OB, Hs, FF, B1f, B2f, RT):
        it = pl.program_id(0)

        def layernorm_rows(r0, nrows):
            x = XR[_ds(r0, nrows, 64), :].astype(F32)
            mu = jnp.mean(x, axis=-1, keepdims=True)
            xc = x - mu
            var = jnp.mean(xc * xc, axis=-1, keepdims=True)
            xn = xc * lax.rsqrt(var + 1e-5)
            XN[_ds(r0, nrows, 64), :] = xn
            nb = nrows // 64
            lo = jnp.concatenate([xn[64 * i:64 * i + 32] for i in range(nb)], axis=0)
            hi = jnp.concatenate([xn[64 * i + 32:64 * i + 64] for i in range(nb)], axis=0)
            XBlo[_ds(r0 // 4, nrows // 4, 16), :] = _pk(lo)
            XBhi[_ds(r0 // 4, nrows // 4, 16), :] = _pk(hi)

        def relayout_piece(p):
            s32 = stg.bitcast(U32)
            blk = s32.at[_ds(p * 256, 256, 256)]
            m = p // 64
            r0 = (p % 64) * 8
            for u in range(2):
                for pp in range(8):
                    A = blk[pl.ds((2 * pp) * 16 + 8 * u, 8), :]
                    B = blk[pl.ds((2 * pp + 1) * 16 + 8 * u, 8), :]
                    lo = (A & 0xFFFF) | (B << 16)
                    hi = (A >> 16) | (B & np.uint32(0xFFFF0000))
                    RT[pl.ds((u * 2) * TR + pp, 8, stride=9), :] = lo
                    RT[pl.ds((u * 2 + 1) * TR + pp, 8, stride=9), :] = hi
            for u in range(2):
                for i in range(8):
                    hp = 8 * u + i
                    for par in range(2):
                        v = RT[pl.ds((u * 2 + par) * TR + 9 * i, 8), :]
                        wqkv[m * H + 2 * hp + par, _ds(r0, 8, 8), :] = v

        @pl.when(it == 0)
        def _prologue():
            sem_i = [0]
            def nsem():
                s_ = sems.at[sem_i[0]]; sem_i[0] += 1
                return s_
            S_X = sem_i[0]
            cx = [pltpu.make_async_copy(x_h.at[pl.ds(i * 512, 512)], XR.at[pl.ds(i * 512, 512)], nsem()) for i in range(4)]
            w1_32 = w1_h.bitcast(U32); w2_32 = w2_h.bitcast(U32); wo_32 = wo_h.bitcast(U32)
            S_W1 = sem_i[0]
            cw1 = [pltpu.make_async_copy(w1_32.at[:, pl.ds(j * 128, 128)], w1.at[j], nsem()) for j in range(FT)]
            S_W2 = sem_i[0]
            cw2 = [pltpu.make_async_copy(w2_32.at[:, pl.ds(j * 128, 128)], w2.at[j], nsem()) for j in range(KT)]
            S_QKV = sem_i[0]
            cq = []
            for m, wh in enumerate((wq_h, wk_h, wv_h)):
                cq.append([pltpu.make_async_copy(wh.at[pl.ds(c * 2048, 2048)],
                                                 stg.at[pl.ds((m * 16 + c) * 2048, 2048)], nsem()) for c in range(16)])
            cwo = [pltpu.make_async_copy(wo_32.at[:, pl.ds(j * 128, 128)], wo.at[j], nsem()) for j in range(KT)]

            with jax.named_scope("P_issue"):
                cx[0].start()
                cx[1].start()
                for c in cw1[0:14]: c.start()
                cx[2].start()
                for c in cw1[14:21]: c.start()
                cx[3].start()
                for c in cw1[21:]: c.start()

            mem_s[...] = mem0_ref[...].astype(F32)
            B1f[...] = b1_ref[...].astype(F32)
            B2f[...] = b2_ref[...].astype(F32)

            with jax.named_scope("P_waitx"):
                cx[0].wait()
            def ln_body(i, _):
                layernorm_rows(i * 128, 128)
                return 0
            with jax.named_scope("P_ln"):
                lax.fori_loop(0, 4, ln_body, 0)
            with jax.named_scope("P_issue2"):
                for c in cq[0]: c.start()
                for c in cw2: c.start()
            with jax.named_scope("P_ln2"):
                cx[1].wait()
                lax.fori_loop(4, 8, ln_body, 0)

            def wait_like(ref, sem):
                pltpu.make_async_copy(ref, ref, sem).wait()

            def spread(nslots, thunks):
                out = [[] for _ in range(nslots)]
                n = len(thunks)
                for i, f in enumerate(thunks):
                    out[(i * nslots) // n].append(f)
                return out

            def p1(b, side):
                def body(g, _):
                    if b == 0:
                        for t in range(7):
                            wait_like(w1.at[0], sems.at[S_W1 + g * 7 + t])
                    sl = spread(14, side(g))
                    for half in range(2):
                        lhs = _bc(XBlo[pl.ds(b * 256 + half * 128, 128), :])
                        for t in range(7):
                            j = g * 7 + t
                            hh = _mm(lhs, _bc(w1[j])) + B1f[pl.ds(j, 1), :]
                            for f in sl[half * 7 + t]:
                                f()
                            Hp[b * 2 + half, :, _ds(j * 128, 128, 128)] = _pk(_gelu(hh))
                    return 0
                lax.fori_loop(0, 4, body, 0)

            KC = opts.get('kc', 4)
            def p2(b, side):
                def body(g, _):
                    sl = spread(4 * KC, side(g))
                    kw = F // KC
                    for half in range(2):
                        for t in range(2):
                            n = g * 2 + t
                            acc = None
                            for c in range(KC):
                                lhs = _bc(Hp[b * 2 + half, :, c * kw:(c + 1) * kw])
                                d = _mm(lhs, _bc(w2[n, c * kw // 2:(c + 1) * kw // 2, :]))
                                acc = d if acc is None else acc + d
                                for f in sl[(half * 2 + t) * KC + c]:
                                    f()
                            ff = acc + B2f[pl.ds(n, 1), :]
                            FFO[pl.ds(b * 512 + half * 256, 256), _ds(n * 128, 128, 128)] = ff
                    return 0
                lax.fori_loop(0, 4, body, 0)

            def side_ln(g):
                @pl.when((g == 1) | (g == 2))
                def _():
                    wait_like(XR.at[pl.ds(0, 512)], sems.at[S_X + 1 + g])
                r0 = jnp.minimum(640 + 384 * g, 1664)
                lnr = opts.get('lnr', 128)
                return [functools.partial(layernorm_rows, r0 + i * lnr, lnr) for i in range(384 // lnr)]

            def side_rl(p0, npc):
                def f(g):
                    for t in range(npc // 4):
                        wait_like(stg.at[pl.ds(0, 2048)], sems.at[S_QKV + (p0 + g * npc) // 4 + t])
                    return [functools.partial(relayout_piece, p0 + g * npc + t) for t in range(npc)]
                return f

            with jax.named_scope("P_p1_0"):
                p1(0, side_ln)
            with jax.named_scope("P_issue3"):
                for c in cq[1]: c.start()
                for c in cq[2]: c.start()
                for c in cwo: c.start()
            with jax.named_scope("P_p1_1"):
                p1(1, side_rl(0, rl[0]))
            for c in cw2: c.wait()
            with jax.named_scope("P_p2_0"):
                p2(0, side_rl(4 * rl[0], rl[1]))
            with jax.named_scope("P_p2_1"):
                p2(1, side_rl(4 * (rl[0] + rl[1]), rl[2]))
            with jax.named_scope("P_wo"):
                for c in cwo: c.wait()

        r64 = it * 64
        _sc = jax.named_scope("MAIN"); _sc.__enter__()
        xnA = XN[_ds(r64, 40, 64), :]
        xnB = XN[_ds(r64 + 40, 24, 8), :]
        xh = _bc(XBhi[_ds(it * 16, 16, 16), :])

        NP = H // 2
        row = lax.broadcasted_iota(jnp.int32, (2 * L, 2 * L), 0)
        col = lax.broadcasted_iota(jnp.int32, (2 * L, 2 * L), 1)
        rowh = jnp.where(row >= L, row - L, row)
        colh = jnp.where(col >= L, col - L, col)
        mask = ((rowh < M) | (rowh >= colh)) & ((row >= L) == (col >= L))
        c2 = scale * 1.4426950408889634

        def qk(q, k):
            return lax.dot_general(q, k, (((1,), (1,)), ((), ())), preferred_element_type=F32)

        def soft(s):
            s = jnp.where(mask, s * c2, -1e30)
            m = jnp.max(s, axis=-1, keepdims=True)
            e = jnp.exp2(s - m)
            l = jnp.sum(e, axis=-1, keepdims=True)
            r = pl.reciprocal(l, approx=True)
            r = r * (2.0 - l * r)
            return e.astype(BF), r

        def ffn1(j):
            hh = _mm(xh, _bc(w1[j])) + B1f[j:j + 1, :]
            Hs[:, j * 128:(j + 1) * 128] = _pk(_gelu(hh))

        def ffn2(j):
            FF[:, j * 128:(j + 1) * 128] = _mm(_bc(Hs[...]), _bc(w2[j])) + B2f[j:j + 1, :]

        def run_pass(lhs, asm, emit, mid, fill):
            st = {}
            def proj2(base, t):
                r0 = asm(_mm(lhs, _bc(wqkv[base + 2 * t])), base + 2 * t)
                r1 = asm(_mm(lhs, _bc(wqkv[base + 2 * t + 1])), base + 2 * t + 1)
                return jnp.concatenate([r0, r1], axis=0).astype(BF)
            for t in range(NP + 2):
                if t < NP:
                    q = proj2(0, t)
                    k = proj2(H, t)
                else:
                    for f in fill[t - NP]:
                        f()
                if 1 <= t <= NP:
                    qq, kk = st[t - 1]['q'], st[t - 1]['k']
                    st[t - 1]['e'], st[t - 1]['r'] = soft(qk(qq, kk))
                if t < NP:
                    v = proj2(2 * H, t)
                    st[t] = dict(q=q, k=k, v=v)
                    for f in mid.get(t, []):
                        f()
                if 2 <= t <= NP + 1:
                    d = st.pop(t - 2)
                    o = _mm(d['e'], d['v']) * d['r']
                    emit(2 * (t - 2), o[0:L])
                    emit(2 * (t - 2) + 1, o[L:2 * L])

        f1 = [functools.partial(ffn1, j) for j in range(FT)]
        n0, n1, n2 = o_f1
        for f in f1[:n0]:
            f()
        mem = mem_s[...]
        lhsA = jnp.concatenate([mem, xnA], axis=0).astype(BF)

        def asmA(r, idx):
            carry[:, idx * 128:(idx + 1) * 128] = r[40:48]
            return r[0:40]

        def emitA(h, o):
            OA[:, h * 128:(h + 1) * 128] = _pk(jnp.concatenate([o[0:8], o[16:40]], axis=0))
            oleft[:, h * 128:(h + 1) * 128] = o[8:16]

        nmid = FT - n0 - n1 - n2
        mid = {}
        for i in range(nmid):
            mid.setdefault((i * NP) // nmid, []).append(f1[n0 + i])
        a0 = n0 + nmid
        run_pass(lhsA, asmA, emitA, mid, [f1[a0:a0 + n1 // 2], f1[a0 + n1 // 2:a0 + n1]])
        outA = []
        for j in range(KT):
            outA.append(_mm(_bc(OA[...]), _bc(wo[j])))
        memB = jnp.concatenate([a[0:8] for a in outA], axis=1)
        for f in f1[a0 + n1:]:
            f()

        lhsB = jnp.concatenate([memB, xnB], axis=0).astype(BF)
        z8 = jnp.zeros((8, 128), F32)

        def asmB(r, idx):
            return jnp.concatenate([r[0:8], carry[:, idx * 128:(idx + 1) * 128], r[8:32]], axis=0)

        def emitB(h, o):
            OB[:, h * 128:(h + 1) * 128] = _pk(jnp.concatenate(
                [o[0:8], oleft[:, h * 128:(h + 1) * 128], o[8:40]], axis=0))

        run_pass(lhsB, asmB, emitB, {}, [[functools.partial(ffn2, 0)], [functools.partial(ffn2, 1)]])
        for j in range(KT):
            ob = _mm(_bc(OB[...]), _bc(wo[j]))
            if j + 2 < KT:
                ffn2(j + 2)
            mem_s[:, j * 128:(j + 1) * 128] = ob[0:8]
            a = outA[j]
            att = jnp.concatenate([ob[8:16], a[8:32], ob[16:48]], axis=0)
            ff = jnp.concatenate([FFO[_ds(it * 32, 32, 32), j * 128:(j + 1) * 128],
                                  FF[:, j * 128:(j + 1) * 128]], axis=0)
            xr = XR[_ds(r64, 64, 64), j * 128:(j + 1) * 128].astype(F32)
            res = xr + att + ff
            o_ref[:, j * 128:(j + 1) * 128] = res.astype(BF)
        _sc.__exit__(None, None, None)

    scratch = [
        pltpu.VMEM((3 * H, Dm // 2, 128), U32),
        pltpu.VMEM((KT, HD // 2, 128), U32),
        pltpu.VMEM((FT, Dm // 2, 128), U32),
        pltpu.VMEM((KT, F // 2, 128), U32),
        pltpu.VMEM((3 * Dm * H, 128), BF),
        pltpu.VMEM((S, Dm), BF),
        pltpu.VMEM((S, Dm), F32),
        pltpu.VMEM((S // 4, Dm), U32),
        pltpu.VMEM((S // 4, Dm), U32),
        pltpu.VMEM((4, 128, F), U32),
        pltpu.VMEM((S // 2, Dm), F32),
        pltpu.SemaphoreType.DMA((4 + FT + KT + 48 + KT,)),
        pltpu.VMEM((M, Dm), F32),
        pltpu.VMEM((8, 3 * HD), F32),
        pltpu.VMEM((8, HD), F32),
        pltpu.VMEM((16, HD), U32),
        pltpu.VMEM((24, HD), U32),
        pltpu.VMEM((16, F), U32),
        pltpu.VMEM((32, Dm), F32),
        pltpu.VMEM((FT, 128), F32),
        pltpu.VMEM((KT, 128), F32),
        pltpu.VMEM((4 * TR, 128), U32),
    ]
    return kernel, scratch


@functools.partial(jax.jit, static_argnames=("A_seg_len",))
def pallas_parallel_sum__memory_aug_recurrent_mem_tr__dense_activation_gelu__prompt_kernel(A_x, A_mem0, A_Wq, A_Wk, A_Wv, A_Wo, A_seg_len, B_x, B_w1, B_b1, B_w2, B_b2):
    Bn, S, Dm = A_x.shape
    _, H, Dh = A_Wq.shape
    M = A_mem0.shape[1]
    F = B_w1.shape[1]
    seg = A_seg_len
    kernel, scratch = make_kernel(S, Dm, H, Dh, M, seg, F, {"lnr":64})
    TB = 2 * seg
    any_spec = pl.BlockSpec(memory_space=pl.ANY)
    out = pl.pallas_call(
        kernel,
        grid=(S // TB,),
        in_specs=[
            pl.BlockSpec((M, Dm), lambda i: (0, 0)),
            pl.BlockSpec((F // 128, 128), lambda i: (0, 0)),
            pl.BlockSpec((Dm // 128, 128), lambda i: (0, 0)),
            any_spec, any_spec, any_spec, any_spec, any_spec, any_spec, any_spec,
        ],
        out_specs=pl.BlockSpec((TB, Dm), lambda i: (i, 0)),
        out_shape=jax.ShapeDtypeStruct((S, Dm), A_x.dtype),
        scratch_shapes=scratch,
        compiler_params=pltpu.CompilerParams(
            dimension_semantics=("arbitrary",),
            vmem_limit_bytes=120 * 1024 * 1024),
    )(A_mem0.reshape(M, Dm), B_b1.reshape(F // 128, 128), B_b2.reshape(Dm // 128, 128),
      A_x.reshape(S, Dm),
      A_Wq.reshape(Dm * H, Dh), A_Wk.reshape(Dm * H, Dh), A_Wv.reshape(Dm * H, Dh),
      A_Wo.reshape(H * Dh, Dm), B_w1, B_w2)
    return out.reshape(Bn, S, Dm)
```

```python
import functools
import jax, jax.numpy as jnp, numpy as np
from jax import lax
from jax.experimental import pallas as pl
from jax.experimental.pallas import tpu as pltpu

BF = jnp.bfloat16
F32 = jnp.float32
U32 = jnp.uint32

import contextlib
_USE_SCOPES = False
def _scope(name):
    return jax.named_scope(name) if _USE_SCOPES else contextlib.nullcontext()

def _bc(x):
    return pltpu.bitcast(x, BF)

def _pk(x):
    return pltpu.bitcast(x.astype(BF), U32)

def _mm(a, b):
    return jnp.dot(a, b, preferred_element_type=F32)

def _gelu(x):
    c = 0.7978845608028654
    return 0.5 * x * (1.0 + jnp.tanh(c * (x + 0.044715 * (x * x * x))))

def _ds(start, size, mult):
    if isinstance(start, int):
        return pl.ds(start, size)
    return pl.ds(pl.multiple_of(start, mult), size)

def make_kernel(S, Dm, H, Dh, M, seg, F, opts):
    KT = Dm // 128
    FT = F // 128
    HD = H * Dh
    scale = float(Dh) ** -0.5
    L = M + seg
    NIT = S // 64
    TR = 72
    unr = opts.get('unr', 1)
    pin = opts.get('pin', 1)
    pin2 = opts.get('pin2', 0)
    SUB = opts.get('sub', 1)
    rl = opts.get('rl', [4, 24, 20])
    assert sum(rl) * 4 == 192
    full = opts.get('full', False)
    MB1 = opts.get('mb1', 256)
    MB2 = opts.get('mb2', 256)
    o_f1 = tuple(opts.get('f1', (1, 8, 8)))

    def kernel(mem0_h, b1_h, b2_h, x_h, wq_h, wk_h, wv_h, wo_h, w1_h, w2_h,
               o_ref,
               wqkv, wo, w1, w2, stg, XR, XN, XBlo0, XBlo1, XBhi, Hp, FFO, sems,
               mem_s, carry, oleft, OA, OB, Hs, FF, B1f, B2f, RT, mem0_ref, b1_ref, b2_ref, ZM):
        it = pl.program_id(0)

        LNR = opts.get('lnp', 16)

        def layernorm_part(blk, part, sblk=None, upper=False):
            sblk = blk if sblk is None else sblk
            x = XR[_ds(sblk * 64 + part * LNR, LNR, LNR), :].astype(F32)
            mu = jnp.mean(x, axis=-1, keepdims=True)
            xc = x - mu
            var = jnp.mean(xc * xc, axis=-1, keepdims=True)
            xn = xc * lax.rsqrt(var + 1e-5)
            XN[_ds(blk * 64 + part * LNR, LNR, LNR), :] = xn
            off = (part * LNR) % 32
            if part * LNR < 32:
                if upper:
                    XBlo1[_ds((blk - 16) * 16 + off // 2, LNR // 2, 8), :] = _pk(xn)
                else:
                    XBlo0[_ds(blk * 16 + off // 2, LNR // 2, 8), :] = _pk(xn)
            else:
                XBhi[_ds(blk * 16 + off // 2, LNR // 2, 8), :] = _pk(xn)
            if not opts.get('tokall', True):
                return xn[0:8, 0:128]
            bits = pltpu.bitcast(xn, U32)
            acc = None
            for rr in range(LNR // 8):
                for cc in range(KT):
                    v_ = bits[rr * 8:(rr + 1) * 8, cc * 128:(cc + 1) * 128]
                    acc = v_ if acc is None else (acc | v_)
            return pltpu.bitcast(acc, F32)

        def layernorm_block(blk):
            for part in range(64 // LNR):
                layernorm_part(blk, part)

        def relayout_piece(p):
            s32 = stg.bitcast(U32)
            blk = s32.at[_ds(p * 256, 256, 256)]
            m = p // 64
            r0 = (p % 64) * 8
            for u in range(2):
                for pp in range(8):
                    A = blk[pl.ds((2 * pp) * 16 + 8 * u, 8), :]
                    B = blk[pl.ds((2 * pp + 1) * 16 + 8 * u, 8), :]
                    lo = (A & 0xFFFF) | (B << 16)
                    hi = (A >> 16) | (B & np.uint32(0xFFFF0000))
                    RT[pl.ds((u * 2) * TR + pp, 8, stride=9), :] = lo
                    RT[pl.ds((u * 2 + 1) * TR + pp, 8, stride=9), :] = hi
            tok = None
            for u in range(2):
                for i in range(8):
                    hp = 8 * u + i
                    for par in range(2):
                        v = RT[pl.ds((u * 2 + par) * TR + 9 * i, 8), :]
                        wqkv[m * H + 2 * hp + par, _ds(r0, 8, 8), :] = v
                        if opts.get('rltok', 1) == 2 or i == 7:
                            tok = v if tok is None else (tok | v)
            return pltpu.bitcast(tok, F32) if pin2 else None

        @pl.when(it == 0)
        def _prologue():
            sem_i = [0]
            def nsem():
                s_ = sems.at[sem_i[0]]; sem_i[0] += 1
                return s_
            S_X = sem_i[0]
            cx = [pltpu.make_async_copy(x_h.at[pl.ds(i * 512, 512)], XR.at[pl.ds(i * 512, 512)], nsem()) for i in range(4)]
            w1_32 = w1_h.bitcast(U32); w2_32 = w2_h.bitcast(U32); wo_32 = wo_h.bitcast(U32)
            S_W1 = sem_i[0]
            cw1 = [pltpu.make_async_copy(w1_32.at[:, pl.ds(j * 128, 128)], w1.at[j], nsem()) for j in range(FT)]
            S_W2 = sem_i[0]
            cw2 = [pltpu.make_async_copy(w2_32.at[:, pl.ds(j * 128, 128)], w2.at[j], nsem()) for j in range(KT)]
            S_QKV = sem_i[0]
            cq = []
            for m, wh in enumerate((wq_h, wk_h, wv_h)):
                cq.append([pltpu.make_async_copy(wh.at[pl.ds(c * 2048, 2048)],
                                                 stg.at[pl.ds((m * 16 + c) * 2048, 2048)], nsem()) for c in range(16)])
            cwo = [pltpu.make_async_copy(wo_32.at[:, pl.ds(j * 128, 128)], wo.at[j], nsem()) for j in range(KT)]

            csm = [pltpu.make_async_copy(h_, v_, nsem()) for h_, v_ in ((mem0_h, mem0_ref), (b1_h, b1_ref), (b2_h, b2_ref))]
            with _scope("P_issue"):
                cx[0].start()
                for c in csm: c.start()
                cx[1].start()
                for c in cw1[0:14]: c.start()
                cx[2].start()
                for c in cw1[14:21]: c.start()
                cx[3].start()
                for c in cw1[21:]: c.start()


            with _scope("P_waitx"):
                cx[0].wait()
            def ln_body(i, _):
                layernorm_block(2 * i)
                layernorm_block(2 * i + 1)
                return 0
            with _scope("P_ln"):
                lax.fori_loop(0, 4, ln_body, 0)
            for c in csm: c.wait()
            ZM[...] = jnp.zeros((8, 128), U32)
            mem_s[...] = mem0_ref[...].astype(F32)
            B1f[...] = b1_ref[...].astype(F32)
            B2f[...] = b2_ref[...].astype(F32)
            with _scope("P_issue2"):
                for c in cq[0]: c.start()
                for c in cw2: c.start()
            with _scope("P_ln2"):
                cx[1].wait()
                lax.fori_loop(4, 8, ln_body, 0)

            def wait_like(ref, sem):
                pltpu.make_async_copy(ref, ref, sem).wait()

            def spread(nslots, thunks):
                out = [[] for _ in range(nslots)]
                n = len(thunks)
                for i, f in enumerate(thunks):
                    out[(i * nslots) // n].append(f)
                return out

            def p1(b, side):
                def body(g, _):
                    if b == 0:
                        for t in range(7):
                            wait_like(w1.at[0], sems.at[S_W1 + g * 7 + t])
                    sl = spread(14 - pin, side(g)) + [[]] * pin
                    toks = {}
                    for half in range(2):
                        lhs = _bc((XBlo0, XBlo1)[b][pl.ds(half * 128, 128), :])
                        for t in range(7):
                            j = g * 7 + t
                            si = half * 7 + t
                            bias = B1f[pl.ds(j, 1), :]
                            if pin and toks.get(si - pin):
                                z = None
                                for tk in toks[si - pin]:
                                    zz = pltpu.bitcast(tk, U32) & ZM[...]
                                    z = zz if z is None else (z | zz)
                                bias = bias + pltpu.bitcast(z, F32)[0:1, :]
                            hh = _mm(lhs, _bc(w1[j])) + bias
                            toks[si] = [r for r in (f() for f in sl[si]) if r is not None]
                            Hp[b * 2 + half, :, _ds(j * 128, 128, 128)] = _pk(_gelu(hh))
                    return 0
                lax.fori_loop(0, 4, body, 0)

            KC = opts.get('kc', 4)
            def p2(b, side):
                def body(g, _):
                    sl = spread(4 * KC - pin2, side(g)) + [[]] * pin2
                    kw = F // KC
                    toks = {}
                    for half in range(2):
                        for t in range(2):
                            n = g * 2 + t
                            acc = None
                            for c in range(KC):
                                si = (half * 2 + t) * KC + c
                                lhs = _bc(Hp[b * 2 + half, :, c * kw:(c + 1) * kw])
                                d = _mm(lhs, _bc(w2[n, c * kw // 2:(c + 1) * kw // 2, :]))
                                if pin2 and toks.get(si - pin2):
                                    z = None
                                    for tk in toks[si - pin2]:
                                        zz = pltpu.bitcast(tk, U32) & ZM[...]
                                        z = zz if z is None else (z | zz)
                                    d = d + pltpu.bitcast(z, F32)[0:1, :]
                                acc = d if acc is None else acc + d
                                toks[si] = [r for r in (f() for f in sl[si]) if r is not None]
                            ff = acc + B2f[pl.ds(n, 1), :]
                            FFO[pl.ds(b * 512 + half * 256, 256), _ds(n * 128, 128, 128)] = ff
                    return 0
                lax.fori_loop(0, 4, body, 0)

            def side_ln(g):
                @pl.when((g == 1) | (g == 2))
                def _():
                    wait_like(XR.at[pl.ds(0, 512)], sems.at[S_X + 1 + g])
                b0 = jnp.clip(10 + 6 * g, 16, 26)
                s0 = jnp.where(g == 0, 0, b0)
                return [functools.partial(layernorm_part, b0 + i, part, s0 + i, True)
                        for i in range(6) for part in range(64 // LNR)]

            def side_rl(p0, npc):
                def f(g):
                    for t in range(npc // 4):
                        wait_like(stg.at[pl.ds(0, 2048)], sems.at[S_QKV + (p0 + g * npc) // 4 + t])
                    return [functools.partial(relayout_piece, p0 + g * npc + t) for t in range(npc)]
                return f

            with _scope("P_p1_0"):
                p1(0, side_ln)
            with _scope("P_issue3"):
                for c in cq[1]: c.start()
                for c in cq[2]: c.start()
                for c in cwo: c.start()
            with _scope("P_p1_1"):
                p1(1, side_rl(0, rl[0]))
            for c in cw2: c.wait()
            with _scope("P_p2_0"):
                p2(0, side_rl(4 * rl[0], rl[1]))
            with _scope("P_p2_1"):
                p2(1, side_rl(4 * (rl[0] + rl[1]), rl[2]))
            with _scope("P_wo"):
                for c in cwo: c.wait()

        def main_body(it, sub):
            r64 = it * 64
            xnA = XN[_ds(r64, 40, 64), :]
            xnB = XN[_ds(r64 + 40, 24, 8), :]
            xh = _bc(XBhi[_ds(it * 16, 16, 16), :])

            NP = H // 2
            row = lax.broadcasted_iota(jnp.int32, (2 * L, 2 * L), 0)
            col = lax.broadcasted_iota(jnp.int32, (2 * L, 2 * L), 1)
            rowh = jnp.where(row >= L, row - L, row)
            colh = jnp.where(col >= L, col - L, col)
            mask = ((rowh < M) | (rowh >= colh)) & ((row >= L) == (col >= L))
            c2 = scale * 1.4426950408889634

            def qk(q, k):
                return lax.dot_general(q, k, (((1,), (1,)), ((), ())), preferred_element_type=F32)

            def soft(s):
                s = jnp.where(mask, s * c2, -1e30)
                m = jnp.max(s, axis=-1, keepdims=True)
                e = jnp.exp2(s - m)
                l = jnp.sum(e, axis=-1, keepdims=True)
                r = pl.reciprocal(l, approx=True)
                r = r * (2.0 - l * r)
                return e.astype(BF), r

            def ffn1(j):
                hh = _mm(xh, _bc(w1[j])) + B1f[j:j + 1, :]
                Hs[:, j * 128:(j + 1) * 128] = _pk(_gelu(hh))

            def ffn2(j):
                FF[:, j * 128:(j + 1) * 128] = _mm(_bc(Hs[...]), _bc(w2[j])) + B2f[j:j + 1, :]

            def run_pass(lhs, asm, emit, mid, fill):
                st = {}
                def proj2(base, t):
                    r0 = asm(_mm(lhs, _bc(wqkv[base + 2 * t])), base + 2 * t)
                    r1 = asm(_mm(lhs, _bc(wqkv[base + 2 * t + 1])), base + 2 * t + 1)
                    return jnp.concatenate([r0, r1], axis=0).astype(BF)
                for t in range(NP + 2):
                    if t < NP:
                        q = proj2(0, t)
                        k = proj2(H, t)
                    else:
                        for f in fill[t - NP]:
                            f()
                    if 1 <= t <= NP:
                        qq, kk = st[t - 1]['q'], st[t - 1]['k']
                        st[t - 1]['e'], st[t - 1]['r'] = soft(qk(qq, kk))
                    if t < NP:
                        v = proj2(2 * H, t)
                        st[t] = dict(q=q, k=k, v=v)
                        for f in mid.get(t, []):
                            f()
                    if 2 <= t <= NP + 1:
                        d = st.pop(t - 2)
                        o = _mm(d['e'], d['v']) * d['r']
                        emit(2 * (t - 2), o[0:L])
                        emit(2 * (t - 2) + 1, o[L:2 * L])

            f1 = [functools.partial(ffn1, j) for j in range(FT)]
            n0, n1, n2 = o_f1
            for f in f1[:n0]:
                f()
            mem = mem_s[...]
            lhsA = jnp.concatenate([mem, xnA], axis=0).astype(BF)

            def asmA(r, idx):
                carry[:, idx * 128:(idx + 1) * 128] = r[40:48]
                return r[0:40]

            def emitA(h, o):
                OA[:, h * 128:(h + 1) * 128] = _pk(jnp.concatenate([o[0:8], o[16:40]], axis=0))
                oleft[:, h * 128:(h + 1) * 128] = o[8:16]

            nmid = FT - n0 - n1 - n2
            mid = {}
            for i in range(nmid):
                mid.setdefault((i * NP) // nmid, []).append(f1[n0 + i])
            a0 = n0 + nmid
            run_pass(lhsA, asmA, emitA, mid, [f1[a0:a0 + n1 // 2], f1[a0 + n1 // 2:a0 + n1]])
            outA = []
            for j in range(KT):
                outA.append(_mm(_bc(OA[...]), _bc(wo[j])))
            memB = jnp.concatenate([a[0:8] for a in outA], axis=1)
            for f in f1[a0 + n1:]:
                f()

            lhsB = jnp.concatenate([memB, xnB], axis=0).astype(BF)
            z8 = jnp.zeros((8, 128), F32)

            def asmB(r, idx):
                return jnp.concatenate([r[0:8], carry[:, idx * 128:(idx + 1) * 128], r[8:32]], axis=0)

            def emitB(h, o):
                OB[:, h * 128:(h + 1) * 128] = _pk(jnp.concatenate(
                    [o[0:8], oleft[:, h * 128:(h + 1) * 128], o[8:40]], axis=0))

            f2 = [functools.partial(ffn2, j) for j in range(KT)]
            e0, e1, lag = opts.get('f2', (1, 1, 0))
            run_pass(lhsB, asmB, emitB, {}, [f2[0:e0], f2[e0:e0 + e1]])
            nxt = e1 + e0
            for j in range(KT):
                while nxt <= j:
                    f2[nxt](); nxt += 1
                ob = _mm(_bc(OB[...]), _bc(wo[j]))
                if nxt < KT and j >= lag:
                    f2[nxt](); nxt += 1
                mem_s[:, j * 128:(j + 1) * 128] = ob[0:8]
                a = outA[j]
                att = jnp.concatenate([ob[8:16], a[8:32], ob[16:48]], axis=0)
                ff = jnp.concatenate([FFO[_ds(it * 32, 32, 32), j * 128:(j + 1) * 128],
                                      FF[:, j * 128:(j + 1) * 128]], axis=0)
                xr = XR[_ds(r64, 64, 64), j * 128:(j + 1) * 128].astype(F32)
                res = xr + att + ff
                o_ref[sub * 64:(sub + 1) * 64, j * 128:(j + 1) * 128] = res.astype(BF)


        for sub in range(SUB):
            with _scope("MAIN"):
                main_body(pl.program_id(0) * SUB + sub, sub)

    scratch = [
        pltpu.VMEM((3 * H, Dm // 2, 128), U32),
        pltpu.VMEM((KT, HD // 2, 128), U32),
        pltpu.VMEM((FT, Dm // 2, 128), U32),
        pltpu.VMEM((KT, F // 2, 128), U32),
        pltpu.VMEM((3 * Dm * H, 128), BF),
        pltpu.VMEM((S, Dm), BF),
        pltpu.VMEM((S, Dm), F32),
        pltpu.VMEM((S // 8, Dm), U32),
        pltpu.VMEM((S // 8, Dm), U32),
        pltpu.VMEM((S // 4, Dm), U32),
        pltpu.VMEM((4, 128, F), U32),
        pltpu.VMEM((S // 2, Dm), F32),
        pltpu.SemaphoreType.DMA((4 + FT + KT + 48 + KT + 3,)),
        pltpu.VMEM((M, Dm), F32),
        pltpu.VMEM((8, 3 * HD), F32),
        pltpu.VMEM((8, HD), F32),
        pltpu.VMEM((16, HD), U32),
        pltpu.VMEM((24, HD), U32),
        pltpu.VMEM((16, F), U32),
        pltpu.VMEM((32, Dm), F32),
        pltpu.VMEM((FT, 128), F32),
        pltpu.VMEM((KT, 128), F32),
        pltpu.VMEM((4 * TR + 16, 128), U32),
        pltpu.VMEM((M, Dm), BF),
        pltpu.VMEM((FT, 128), BF),
        pltpu.VMEM((KT, 128), BF),
        pltpu.VMEM((8, 128), U32),
    ]
    return kernel, scratch


@functools.partial(jax.jit, static_argnames=("A_seg_len",))
def pallas_parallel_sum__memory_aug_recurrent_mem_tr__dense_activation_gelu__prompt_kernel(A_x, A_mem0, A_Wq, A_Wk, A_Wv, A_Wo, A_seg_len, B_x, B_w1, B_b1, B_w2, B_b2):
    Bn, S, Dm = A_x.shape
    _, H, Dh = A_Wq.shape
    M = A_mem0.shape[1]
    F = B_w1.shape[1]
    seg = A_seg_len
    kernel, scratch = make_kernel(S, Dm, H, Dh, M, seg, F, {})
    TB = 2 * seg * 1
    any_spec = pl.BlockSpec(memory_space=pl.ANY)
    out = pl.pallas_call(
        kernel,
        grid=(S // TB,),
        in_specs=[
            any_spec, any_spec, any_spec,
            any_spec, any_spec, any_spec, any_spec, any_spec, any_spec, any_spec,
        ],
        out_specs=pl.BlockSpec((TB, Dm), lambda i: (i, 0)),
        out_shape=jax.ShapeDtypeStruct((S, Dm), A_x.dtype),
        scratch_shapes=scratch,
        compiler_params=pltpu.CompilerParams(
            dimension_semantics=("arbitrary",),
            vmem_limit_bytes=120 * 1024 * 1024),
    )(A_mem0.reshape(M, Dm), B_b1.reshape(F // 128, 128), B_b2.reshape(Dm // 128, 128),
      A_x.reshape(S, Dm),
      A_Wq.reshape(Dm * H, Dh), A_Wk.reshape(Dm * H, Dh), A_Wv.reshape(Dm * H, Dh),
      A_Wo.reshape(H * Dh, Dm), B_w1, B_w2)
    return out.reshape(Bn, S, Dm)
```

```python
import functools

import jax
import jax.numpy as jnp
import numpy as np
from jax import lax
from jax.experimental import pallas as pl
from jax.experimental.pallas import tpu as pltpu

BF = jnp.bfloat16
F32 = jnp.float32
U32 = jnp.uint32
LOG2E = 1.4426950408889634


def _unpack(x):
    return pltpu.bitcast(x, BF)


def _pack(x):
    return pltpu.bitcast(x.astype(BF), U32)


def _mm(a, b):
    return jnp.dot(a, b, preferred_element_type=F32)


def _gelu(x):
    c = 0.7978845608028654
    return 0.5 * x * (1.0 + jnp.tanh(c * (x + 0.044715 * (x * x * x))))


def _ds(start, size, mult):
    if isinstance(start, int):
        return pl.ds(start, size)
    return pl.ds(pl.multiple_of(start, mult), size)


def _spread(nslots, thunks):
    out = [[] for _ in range(nslots)]
    for i, f in enumerate(thunks):
        out[(i * nslots) // len(thunks)].append(f)
    return out


def _make_kernel(S, Dm, H, Dh, M, seg, F):
    KT = Dm // 128
    FT = F // 128
    HD = H * Dh
    L = M + seg
    NB = S // (2 * seg)
    NP = H // 2
    TR = 72
    c_soft = float(Dh) ** -0.5 * LOG2E
    G1, G2, GL = 3, 8, 5
    NPIECE = 3 * Dm // 16

    S_X, S_SM, S_W1 = 0, 3, 6
    S_W2 = S_W1 + FT
    S_QKV = S_W2 + KT
    S_WO = S_QKV + 48
    S_OUT = S_WO + KT
    NSEM = S_OUT + 1

    def kernel(mem0_h, b1_h, b2_h, x_h, wq_h, wk_h, wv_h, wo_h, w1_h, w2_h,
               o_h,
               wqkv, wo_b, w1_b, w2_b, stg, XR, XN, XBlo0, XBlo1, XBhi, Hp, FFO, sems,
               mem_s, carry, oleft, OA, OB, Hs, FF, B1f, B2f, RT,
               mem0_v, b1_v, b2_v, ZM):
        wo, w1, w2 = wo_b.bitcast(U32), w1_b.bitcast(U32), w2_b.bitcast(U32)

        def wait_like(ref, sem):
            pltpu.make_async_copy(ref, ref, sem).wait()

        def layernorm16(blk, part):
            x = XR[blk, _ds(part * 16, 16, 16), :].astype(F32)
            mu = jnp.mean(x, axis=-1, keepdims=True)
            xc = x - mu
            var = jnp.mean(xc * xc, axis=-1, keepdims=True)
            xn = xc * lax.rsqrt(var + 1e-5)
            XN[_ds(blk * 64 + part * 16, 16, 16), :] = xn
            return xn

        def token(xn):
            bits = pltpu.bitcast(xn, U32)
            acc = None
            for rr in range(xn.shape[0] // 8):
                for cc in range(KT):
                    v_ = bits[rr * 8:(rr + 1) * 8, cc * 128:(cc + 1) * 128]
                    acc = v_ if acc is None else (acc | v_)
            return acc

        def ln_lo(dst, blk, blk0, part):
            xn = layernorm16(blk, part)
            dst[_ds((blk - blk0) * 16 + 8 * part, 8, 8), :] = _pack(xn)
            return xn

        def ln_side_lo(blk, part):
            return token(ln_lo(XBlo1, blk, 16, part))

        def ln_side_hi(blk, part):
            xn = layernorm16(blk, 2 + part)
            XBhi[_ds(blk * 16 + 8 * part, 8, 8), :] = _pack(xn)
            return token(xn)

        def retile_piece(p):
            blk = stg.bitcast(U32).at[_ds(p * 256, 256, 256)]
            m = p // 64
            r0 = (p % 64) * 8
            for u in range(2):
                for pp in range(8):
                    A = blk[pl.ds((2 * pp) * 16 + 8 * u, 8), :]
                    B = blk[pl.ds((2 * pp + 1) * 16 + 8 * u, 8), :]
                    lo = (A & 0xFFFF) | (B << 16)
                    hi = (A >> 16) | (B & np.uint32(0xFFFF0000))
                    RT[pl.ds((u * 2) * TR + 9 * pp, 8), :] = lo
                    RT[pl.ds((u * 2 + 1) * TR + 9 * pp, 8), :] = hi
            for u in range(2):
                for i in range(8):
                    for par in range(2):
                        v = RT[pl.ds((u * 2 + par) * TR + i, 8, stride=9), :]
                        wqkv[m * H + 2 * (8 * u + i) + par, _ds(r0, 8, 8), :] = v

        cxlo = pltpu.make_async_copy(x_h.at[0:16, 0:32], XR.at[0:16, 0:32], sems.at[S_X])
        cx1lo = pltpu.make_async_copy(x_h.at[16:32, 0:32], XR.at[16:32, 0:32], sems.at[S_X + 1])
        cxhi = pltpu.make_async_copy(x_h.at[:, 32:64], XR.at[:, 32:64], sems.at[S_X + 2])
        csm = [pltpu.make_async_copy(h_, v_, sems.at[S_SM + i])
               for i, (h_, v_) in enumerate(((mem0_h, mem0_v), (b1_h, b1_v), (b2_h, b2_v)))]
        cw1 = [pltpu.make_async_copy(w1_h.at[:, pl.ds(j * 128, 128)], w1_b.at[j], sems.at[S_W1 + j])
               for j in range(FT)]
        cw2 = [pltpu.make_async_copy(w2_h.at[:, pl.ds(j * 128, 128)], w2_b.at[j], sems.at[S_W2 + j])
               for j in range(KT)]
        cq = [[pltpu.make_async_copy(wh.at[pl.ds(c * 2048, 2048)],
                                     stg.at[pl.ds((m * 16 + c) * 2048, 2048)],
                                     sems.at[S_QKV + m * 16 + c]) for c in range(16)]
              for m, wh in enumerate((wq_h, wk_h, wv_h))]
        cwo = [pltpu.make_async_copy(wo_h.at[:, pl.ds(j * 128, 128)], wo_b.at[j], sems.at[S_WO + j])
               for j in range(KT)]

        cxlo.start()
        for c in cw1[0:G1]:
            c.start()
        for c in csm:
            c.start()
        for c in cw1[G1:G2 + GL]:
            c.start()
        cx1lo.start()
        for c in cw1[G2 + GL:]:
            c.start()
        cxhi.start()

        cxlo.wait()

        def ln0_body(i, _):
            for bb in range(4):
                for part in range(2):
                    ln_lo(XBlo0, 4 * i + bb, 0, part)
            return 0
        lax.fori_loop(0, 4, ln0_body, 0)
        for c in csm:
            c.wait()
        ZM[...] = jnp.zeros((8, 128), U32)
        mem_s[...] = mem0_v[...].astype(F32)
        B1f[...] = b1_v[...].astype(F32)
        B2f[...] = b2_v[...].astype(F32)
        for c in cq[0]:
            c.start()
        for c in cw2:
            c.start()

        def ffn1_group(b, j0, nt, side):
            src = (XBlo0, XBlo1)[b]
            sl = (_spread(2 * nt - 1, side) + [[]]) if side else [[]] * (2 * nt)
            toks = {}
            for half in range(2):
                lhs = _unpack(src[pl.ds(half * 128, 128), :])
                for t in range(nt):
                    j = j0 + t
                    si = half * nt + t
                    bias = B1f[pl.ds(j, 1), :]
                    if toks.get(si - 1):
                        z = None
                        for tk in toks[si - 1]:
                            z = tk if z is None else (z | tk)
                        bias = bias + pltpu.bitcast(z & ZM[...], F32)[0:1, :]
                    hh = _mm(lhs, _unpack(w1[j])) + bias
                    toks[si] = [r for r in (f() for f in sl[si]) if r is not None]
                    Hp[b * 2 + half, :, _ds(j * 128, 128, 128)] = _pack(_gelu(hh))

        def ffn2_group(b, g, side):
            sl = _spread(4, side)
            for half in range(2):
                for t in range(2):
                    n = g * 2 + t
                    ff = _mm(_unpack(Hp[b * 2 + half]), _unpack(w2[n]))
                    for f in sl[half * 2 + t]:
                        f()
                    FFO[pl.ds(b * 512 + half * 256, 256), _ds(n * 128, 128, 128)] = ff + B2f[pl.ds(n, 1), :]

        def retile_side(p0):
            for t in range(6):
                wait_like(stg.at[pl.ds(0, 2048)], sems.at[S_QKV + p0 // 4 + t])
            return [functools.partial(retile_piece, p0 + t) for t in range(24)]

        for c in cw1[0:G1]:
            c.wait()
        ffn1_group(0, 0, G1, [])
        for c in cw1[G1:G2]:
            c.wait()
        ffn1_group(0, G1, G2 - G1, [])
        cx1lo.wait()

        def p10_body(i, _):
            for t in range(GL):
                wait_like(w1_b.at[0], sems.at[S_W1 + G2 + i * GL + t])
            ffn1_group(0, G2 + i * GL, GL,
                       [functools.partial(ln_side_lo, 16 + 4 * i + k // 2, k % 2) for k in range(8)])
            return 0
        lax.fori_loop(0, 4, p10_body, 0)

        for c in cq[1] + cq[2] + cwo:
            c.start()
        cxhi.wait()

        def p11_body(g, _):
            ffn1_group(1, g * (FT // 2), FT // 2,
                       [functools.partial(ln_side_hi, 16 * g + k // 2, k % 2) for k in range(32)])
            return 0
        lax.fori_loop(0, 2, p11_body, 0)
        for c in cw2:
            c.wait()

        def p20_body(g, _):
            ffn2_group(0, g, retile_side(g * 24))
            return 0
        lax.fori_loop(0, 4, p20_body, 0)

        def p21_body(g, _):
            ffn2_group(1, g, retile_side(NPIECE // 2 + g * 24))
            return 0
        lax.fori_loop(0, 4, p21_body, 0)
        for c in cwo:
            c.wait()

        def main_body(it):
            r64 = it * 64
            xnA = XN[_ds(r64, 40, 64), :]
            xnB = XN[_ds(r64 + 40, 24, 8), :]
            xh = _unpack(XBhi[_ds(it * 16, 16, 16), :])

            row = lax.broadcasted_iota(jnp.int32, (2 * L, 2 * L), 0)
            col = lax.broadcasted_iota(jnp.int32, (2 * L, 2 * L), 1)
            rowh = jnp.where(row >= L, row - L, row)
            colh = jnp.where(col >= L, col - L, col)
            same = (row >= L) == (col >= L)
            keep = ((rowh < M) | (rowh >= colh)) & same
            fill = jnp.where(same, -1e9 * LOG2E, -1e30)

            def softmax_parts(q, k):
                s = lax.dot_general(q, k, (((1,), (1,)), ((), ())), preferred_element_type=F32)
                s = jnp.where(keep, s * c_soft, fill)
                m = jnp.max(s, axis=-1, keepdims=True)
                e = jnp.exp2(s - m)
                l = jnp.sum(e, axis=-1, keepdims=True)
                r = pl.reciprocal(l, approx=True)
                r = r * (2.0 - l * r)
                return e.astype(BF), r

            def ffn1(j):
                hh = _mm(xh, _unpack(w1[j])) + B1f[j:j + 1, :]
                Hs[:, j * 128:(j + 1) * 128] = _pack(_gelu(hh))

            def ffn2(j):
                FF[:, j * 128:(j + 1) * 128] = _mm(_unpack(Hs[...]), _unpack(w2[j])) + B2f[j:j + 1, :]

            def run_pass(lhs, asm, emit, mid, fill_work):
                st = {}

                def proj2(base, t):
                    r0 = asm(_mm(lhs, _unpack(wqkv[base + 2 * t])), base + 2 * t)
                    r1 = asm(_mm(lhs, _unpack(wqkv[base + 2 * t + 1])), base + 2 * t + 1)
                    return jnp.concatenate([r0, r1], axis=0).astype(BF)

                for t in range(NP + 2):
                    if t < NP:
                        q = proj2(0, t)
                    else:
                        for f in fill_work[t - NP]:
                            f()
                    if 1 <= t <= NP:
                        st[t - 1]['e'], st[t - 1]['r'] = softmax_parts(st[t - 1]['q'], st[t - 1]['k'])
                    if t < NP:
                        k = proj2(H, t)
                        v = proj2(2 * H, t)
                        st[t] = dict(q=q, k=k, v=v)
                        for f in mid.get(t, []):
                            f()
                    if 2 <= t <= NP + 1:
                        d = st.pop(t - 2)
                        o = _mm(d['e'], d['v']) * d['r']
                        emit(2 * (t - 2), o[0:L])
                        emit(2 * (t - 2) + 1, o[L:2 * L])

            f1 = [functools.partial(ffn1, j) for j in range(FT)]
            f1[0]()
            lhsA = jnp.concatenate([mem_s[...], xnA], axis=0).astype(BF)

            def asmA(r, idx):
                carry[:, idx * 128:(idx + 1) * 128] = r[L:L + 8]
                return r[0:L]

            def emitA(h, o):
                OA[:, h * 128:(h + 1) * 128] = _pack(jnp.concatenate([o[0:8], o[16:40]], axis=0))
                oleft[:, h * 128:(h + 1) * 128] = o[8:16]

            nmid = FT - 17
            mid = {}
            for i in range(nmid):
                mid.setdefault((i * NP) // nmid, []).append(f1[1 + i])
            a0 = 1 + nmid
            run_pass(lhsA, asmA, emitA, mid, [f1[a0:a0 + 4], f1[a0 + 4:a0 + 8]])
            outA = [_mm(_unpack(OA[...]), _unpack(wo[j])) for j in range(KT)]
            memB = jnp.concatenate([a[0:8] for a in outA], axis=1)
            for f in f1[a0 + 8:]:
                f()

            lhsB = jnp.concatenate([memB, xnB], axis=0).astype(BF)

            def asmB(r, idx):
                return jnp.concatenate([r[0:8], carry[:, idx * 128:(idx + 1) * 128], r[8:32]], axis=0)

            def emitB(h, o):
                OB[:, h * 128:(h + 1) * 128] = _pack(jnp.concatenate(
                    [o[0:8], oleft[:, h * 128:(h + 1) * 128], o[8:40]], axis=0))

            f2 = [functools.partial(ffn2, j) for j in range(KT)]
            run_pass(lhsB, asmB, emitB, {}, [f2[0:1], f2[1:2]])
            for j in range(KT):
                cols = slice(j * 128, (j + 1) * 128)
                ob = _mm(_unpack(OB[...]), _unpack(wo[j]))
                if j + 2 < KT:
                    f2[j + 2]()
                mem_s[:, cols] = ob[0:8]
                att = jnp.concatenate([ob[8:16], outA[j][8:32], ob[16:48]], axis=0)
                ff = jnp.concatenate([FFO[_ds(it * 32, 32, 32), cols], FF[:, cols]], axis=0)
                xr = XR[it, :, cols].astype(F32)
                XR[it, :, cols] = (xr + att + ff).astype(BF)

        def loop_body(it, _):
            main_body(it)
            pltpu.make_async_copy(XR.at[it], o_h.at[it], sems.at[S_OUT]).start()
            return 0
        lax.fori_loop(0, NB, loop_body, 0, unroll=2)
        pltpu.make_async_copy(XR, o_h, sems.at[S_OUT]).wait()

    scratch = [
        pltpu.VMEM((3 * H, Dm // 2, 128), U32),
        pltpu.VMEM((KT, HD, 128), BF),
        pltpu.VMEM((FT, Dm, 128), BF),
        pltpu.VMEM((KT, F, 128), BF),
        pltpu.VMEM((3 * Dm * H, Dh), BF),
        pltpu.VMEM((NB, 64, Dm), BF),
        pltpu.VMEM((S, Dm), F32),
        pltpu.VMEM((S // 8, Dm), U32),
        pltpu.VMEM((S // 8, Dm), U32),
        pltpu.VMEM((S // 4, Dm), U32),
        pltpu.VMEM((4, 128, F), U32),
        pltpu.VMEM((S // 2, Dm), F32),
        pltpu.SemaphoreType.DMA((NSEM,)),
        pltpu.VMEM((M, Dm), F32),
        pltpu.VMEM((8, 3 * HD), F32),
        pltpu.VMEM((8, HD), F32),
        pltpu.VMEM((16, HD), U32),
        pltpu.VMEM((24, HD), U32),
        pltpu.VMEM((16, F), U32),
        pltpu.VMEM((32, Dm), F32),
        pltpu.VMEM((FT, 128), F32),
        pltpu.VMEM((KT, 128), F32),
        pltpu.VMEM((4 * TR + 16, 128), U32),
        pltpu.VMEM((M, Dm), BF),
        pltpu.VMEM((FT, 128), BF),
        pltpu.VMEM((KT, 128), BF),
        pltpu.VMEM((8, 128), U32),
    ]
    return kernel, scratch


@functools.partial(jax.jit, static_argnames=("A_seg_len",))
def pallas_parallel_sum__memory_aug_recurrent_mem_tr__dense_activation_gelu__prompt_kernel(
    A_x, A_mem0, A_Wq, A_Wk, A_Wv, A_Wo, A_seg_len, B_x, B_w1, B_b1, B_w2, B_b2,
):
    del B_x
    Bn, S, Dm = A_x.shape
    _, H, Dh = A_Wq.shape
    M = A_mem0.shape[1]
    F = B_w1.shape[1]
    assert (Bn, S, Dm, H, Dh, M, A_seg_len, F) == (1, 2048, 1024, 32, 128, 8, 32, 3584)
    kernel, scratch = _make_kernel(S, Dm, H, Dh, M, A_seg_len, F)
    any_spec = pl.BlockSpec(memory_space=pl.ANY)
    out = pl.pallas_call(
        kernel,
        grid=(1,),
        in_specs=[any_spec] * 10,
        out_specs=any_spec,
        out_shape=jax.ShapeDtypeStruct((S // 64, 64, Dm), A_x.dtype),
        scratch_shapes=scratch,
        compiler_params=pltpu.CompilerParams(
            dimension_semantics=("arbitrary",),
            vmem_limit_bytes=120 * 1024 * 1024),
    )(A_mem0.reshape(M, Dm), B_b1.reshape(F // 128, 128), B_b2.reshape(Dm // 128, 128),
      A_x.reshape(S // 64, 64, Dm),
      A_Wq.reshape(Dm * H, Dh), A_Wk.reshape(Dm * H, Dh), A_Wv.reshape(Dm * H, Dh),
      A_Wo.reshape(H * Dh, Dm), B_w1, B_w2)
    return out.reshape(Bn, S, Dm)
```

```python
import functools

import jax
import jax.numpy as jnp
import numpy as np
from jax import lax
from jax.experimental import pallas as pl
from jax.experimental.pallas import tpu as pltpu

BF = jnp.bfloat16
F32 = jnp.float32
U32 = jnp.uint32
LOG2E = 1.4426950408889634


def _unpack(x):
    return pltpu.bitcast(x, BF)


def _pack(x):
    return pltpu.bitcast(x.astype(BF), U32)


def _mm(a, b):
    return jnp.dot(a, b, preferred_element_type=F32)


def _gelu(x):
    c = 0.7978845608028654
    return 0.5 * x * (1.0 + jnp.tanh(c * (x + 0.044715 * (x * x * x))))


def _ds(start, size, mult):
    if isinstance(start, int):
        return pl.ds(start, size)
    return pl.ds(pl.multiple_of(start, mult), size)


def _spread(nslots, thunks):
    out = [[] for _ in range(nslots)]
    for i, f in enumerate(thunks):
        out[(i * nslots) // len(thunks)].append(f)
    return out


def _make_kernel(S, Dm, H, Dh, M, seg, F):
    KT = Dm // 128
    FT = F // 128
    HD = H * Dh
    L = M + seg
    NB = S // (2 * seg)
    NP = H // 2
    TR = 72
    c_soft = float(Dh) ** -0.5 * LOG2E
    G1, G2, GL = 3, 8, 5

    S_X, S_SM, S_W1 = 0, 3, 6
    S_W2 = S_W1 + FT
    S_QKV = S_W2 + KT
    S_WO = S_QKV + 48
    S_OUT = S_WO + KT
    NSEM = S_OUT + 1

    def kernel(mem0_h, b1_h, b2_h, x_h, wq_h, wk_h, wv_h, wo_h, w1_h, w2_h,
               o_h,
               wqkv, wo_b, w1_b, w2_b, stg, XR, XN, XBlo0, XBlo1, XBhi, Hp, FFO, sems,
               mem_s, carry, oleft, OA, OB, Hs, FF, B1f, B2f, RT,
               mem0_v, b1_v, b2_v, ZM):
        wo, w1, w2 = wo_b.bitcast(U32), w1_b.bitcast(U32), w2_b.bitcast(U32)

        def wait_like(ref, sem):
            pltpu.make_async_copy(ref, ref, sem).wait()

        def layernorm16(blk, part):
            x = XR[blk, _ds(part * 16, 16, 16), :].astype(F32)
            mu = jnp.mean(x, axis=-1, keepdims=True)
            xc = x - mu
            var = jnp.mean(xc * xc, axis=-1, keepdims=True)
            xn = xc * lax.rsqrt(var + 1e-5)
            XN[_ds(blk * 64 + part * 16, 16, 16), :] = xn
            return xn

        def token(xn):
            bits = pltpu.bitcast(xn, U32)
            acc = None
            for rr in range(xn.shape[0] // 8):
                for cc in range(KT):
                    v_ = bits[rr * 8:(rr + 1) * 8, cc * 128:(cc + 1) * 128]
                    acc = v_ if acc is None else (acc | v_)
            return acc

        def ln_lo(dst, blk, blk0, part):
            xn = layernorm16(blk, part)
            dst[_ds((blk - blk0) * 16 + 8 * part, 8, 8), :] = _pack(xn)
            return xn

        def ln_side_lo(blk, part):
            return token(ln_lo(XBlo1, blk, 16, part))

        def ln_side_hi(blk, part):
            xn = layernorm16(blk, 2 + part)
            XBhi[_ds(blk * 16 + 8 * part, 8, 8), :] = _pack(xn)
            return token(xn)

        def retile_store(p, buf):
            blk = stg.bitcast(U32).at[_ds(p * 256, 256, 256)]
            for u in range(2):
                for pp in range(8):
                    A = blk[pl.ds((2 * pp) * 16 + 8 * u, 8), :]
                    B = blk[pl.ds((2 * pp + 1) * 16 + 8 * u, 8), :]
                    lo = (A & 0xFFFF) | (B << 16)
                    hi = (A >> 16) | (B & np.uint32(0xFFFF0000))
                    RT[pl.ds((buf * 4 + u * 2) * TR + 9 * pp, 8), :] = lo
                    RT[pl.ds((buf * 4 + u * 2 + 1) * TR + 9 * pp, 8), :] = hi

        def retile_load(p, buf):
            m = p // 64
            r0 = (p % 64) * 8
            for u in range(2):
                for i in range(8):
                    for par in range(2):
                        v = RT[pl.ds((buf * 4 + u * 2 + par) * TR + i, 8, stride=9), :]
                        wqkv[m * H + 2 * (8 * u + i) + par, _ds(r0, 8, 8), :] = v

        cxlo = pltpu.make_async_copy(x_h.at[0:16, 0:32], XR.at[0:16, 0:32], sems.at[S_X])
        cx1lo = pltpu.make_async_copy(x_h.at[16:32, 0:32], XR.at[16:32, 0:32], sems.at[S_X + 1])
        cxhi = pltpu.make_async_copy(x_h.at[:, 32:64], XR.at[:, 32:64], sems.at[S_X + 2])
        csm = [pltpu.make_async_copy(h_, v_, sems.at[S_SM + i])
               for i, (h_, v_) in enumerate(((mem0_h, mem0_v), (b1_h, b1_v), (b2_h, b2_v)))]
        cw1 = [pltpu.make_async_copy(w1_h.at[:, pl.ds(j * 128, 128)], w1_b.at[j], sems.at[S_W1 + j])
               for j in range(FT)]
        cw2 = [pltpu.make_async_copy(w2_h.at[:, pl.ds(j * 128, 128)], w2_b.at[j], sems.at[S_W2 + j])
               for j in range(KT)]
        cq = [[pltpu.make_async_copy(wh.at[pl.ds(c * 2048, 2048)],
                                     stg.at[pl.ds((m * 16 + c) * 2048, 2048)],
                                     sems.at[S_QKV + m * 16 + c]) for c in range(16)]
              for m, wh in enumerate((wq_h, wk_h, wv_h))]
        cwo = [pltpu.make_async_copy(wo_h.at[:, pl.ds(j * 128, 128)], wo_b.at[j], sems.at[S_WO + j])
               for j in range(KT)]

        cxlo.start()
        for c in cw1[0:G1]:
            c.start()
        for c in csm:
            c.start()
        for c in cw1[G1:G2 + GL]:
            c.start()
        cx1lo.start()
        for c in cw1[G2 + GL:]:
            c.start()
        cxhi.start()

        cxlo.wait()

        def ln0_body(i, _):
            for bb in range(4):
                for part in range(2):
                    ln_lo(XBlo0, 4 * i + bb, 0, part)
            return 0
        lax.fori_loop(0, 4, ln0_body, 0)
        for c in csm:
            c.wait()
        ZM[...] = jnp.zeros((8, 128), U32)
        mem_s[...] = mem0_v[...].astype(F32)
        B1f[...] = b1_v[...].astype(F32)
        B2f[...] = b2_v[...].astype(F32)
        for c in cq[0]:
            c.start()
        for c in cw2:
            c.start()

        def ffn1_group(b, j0, nt, side):
            src = (XBlo0, XBlo1)[b]
            sl = (_spread(2 * nt - 1, side) + [[]]) if side else [[]] * (2 * nt)
            toks = {}
            for half in range(2):
                lhs = _unpack(src[pl.ds(half * 128, 128), :])
                for t in range(nt):
                    j = j0 + t
                    si = half * nt + t
                    bias = B1f[pl.ds(j, 1), :]
                    if toks.get(si - 1):
                        z = None
                        for tk in toks[si - 1]:
                            z = tk if z is None else (z | tk)
                        bias = bias + pltpu.bitcast(z & ZM[...], F32)[0:1, :]
                    hh = _mm(lhs, _unpack(w1[j])) + bias
                    toks[si] = [r for r in (f() for f in sl[si]) if r is not None]
                    Hp[b * 2 + half, :, _ds(j * 128, 128, 128)] = _pack(_gelu(hh))

        def ffn2_group(b, g, side):
            sl = _spread(4, side)
            for half in range(2):
                for t in range(2):
                    n = g * 2 + t
                    ff = _mm(_unpack(Hp[b * 2 + half]), _unpack(w2[n]))
                    for f in sl[half * 2 + t]:
                        f()
                    FFO[_ds(b * 512 + half * 256, 256, 256), _ds(n * 128, 128, 128)] = ff + B2f[pl.ds(n, 1), :]

        def retile_side(p0):
            for t in range(6):
                wait_like(stg.at[pl.ds(0, 2048)], sems.at[S_QKV + p0 // 4 + t])

            def step(t):
                def f():
                    if t < 24:
                        retile_store(p0 + t, t % 2)
                    if t >= 1:
                        retile_load(p0 + t - 1, (t - 1) % 2)
                return f
            return [step(t) for t in range(25)]

        for c in cw1[0:G1]:
            c.wait()
        ffn1_group(0, 0, G1, [])
        for c in cw1[G1:G2]:
            c.wait()
        ffn1_group(0, G1, G2 - G1, [])
        cx1lo.wait()

        def p10_body(i, _):
            for t in range(GL):
                wait_like(w1_b.at[0], sems.at[S_W1 + G2 + i * GL + t])
            ffn1_group(0, G2 + i * GL, GL,
                       [functools.partial(ln_side_lo, 16 + 4 * i + k // 2, k % 2) for k in range(8)])
            return 0
        lax.fori_loop(0, 4, p10_body, 0)

        for c in cq[1] + cq[2] + cwo:
            c.start()
        cxhi.wait()

        def p11_body(g, _):
            ffn1_group(1, g * (FT // 2), FT // 2,
                       [functools.partial(ln_side_hi, 16 * g + k // 2, k % 2) for k in range(32)])
            return 0
        lax.fori_loop(0, 2, p11_body, 0)
        for c in cw2:
            c.wait()

        def p2_body(i, _):
            ffn2_group(i // 4, i % 4, retile_side(i * 24))
            return 0
        lax.fori_loop(0, 8, p2_body, 0)
        for c in cwo:
            c.wait()

        def main_body(it):
            r64 = it * 64
            xnA = XN[_ds(r64, 40, 64), :]
            xnB = XN[_ds(r64 + 40, 24, 8), :]
            xh = _unpack(XBhi[_ds(it * 16, 16, 16), :])

            row = lax.broadcasted_iota(jnp.int32, (2 * L, 2 * L), 0)
            col = lax.broadcasted_iota(jnp.int32, (2 * L, 2 * L), 1)
            rowh = jnp.where(row >= L, row - L, row)
            colh = jnp.where(col >= L, col - L, col)
            same = (row >= L) == (col >= L)
            keep = ((rowh < M) | (rowh >= colh)) & same
            fill = jnp.where(same, -1e9 * LOG2E, -1e30)

            def softmax_parts(q, k):
                s = lax.dot_general(q, k, (((1,), (1,)), ((), ())), preferred_element_type=F32)
                s = jnp.where(keep, s * c_soft, fill)
                m = jnp.max(s, axis=-1, keepdims=True)
                e = jnp.exp2(s - m)
                l = jnp.sum(e, axis=-1, keepdims=True)
                r = pl.reciprocal(l, approx=True)
                r = r * (2.0 - l * r)
                return e.astype(BF), r

            def ffn1(j):
                hh = _mm(xh, _unpack(w1[j])) + B1f[j:j + 1, :]
                Hs[:, j * 128:(j + 1) * 128] = _pack(_gelu(hh))

            def ffn2(j):
                FF[:, j * 128:(j + 1) * 128] = _mm(_unpack(Hs[...]), _unpack(w2[j])) + B2f[j:j + 1, :]

            def run_pass(lhs, asm, emit, mid, fill_work):
                st = {}

                def proj2(base, t):
                    r0 = asm(_mm(lhs, _unpack(wqkv[base + 2 * t])), base + 2 * t)
                    r1 = asm(_mm(lhs, _unpack(wqkv[base + 2 * t + 1])), base + 2 * t + 1)
                    return jnp.concatenate([r0, r1], axis=0).astype(BF)

                for t in range(NP + 2):
                    if t < NP:
                        q = proj2(0, t)
                    else:
                        for f in fill_work[t - NP]:
                            f()
                    if 1 <= t <= NP:
                        st[t - 1]['e'], st[t - 1]['r'] = softmax_parts(st[t - 1]['q'], st[t - 1]['k'])
                    if t < NP:
                        k = proj2(H, t)
                        v = proj2(2 * H, t)
                        st[t] = dict(q=q, k=k, v=v)
                        for f in mid.get(t, []):
                            f()
                    if 2 <= t <= NP + 1:
                        d = st.pop(t - 2)
                        o = _mm(d['e'], d['v']) * d['r']
                        emit(2 * (t - 2), o[0:L])
                        emit(2 * (t - 2) + 1, o[L:2 * L])

            f1 = [functools.partial(ffn1, j) for j in range(FT)]
            f1[0]()
            lhsA = jnp.concatenate([mem_s[...], xnA], axis=0).astype(BF)

            def asmA(r, idx):
                carry[:, idx * 128:(idx + 1) * 128] = r[L:L + 8]
                return r[0:L]

            def emitA(h, o):
                OA[:, h * 128:(h + 1) * 128] = _pack(jnp.concatenate([o[0:8], o[16:40]], axis=0))
                oleft[:, h * 128:(h + 1) * 128] = o[8:16]

            nmid = FT - 17
            mid = {}
            for i in range(nmid):
                mid.setdefault((i * NP) // nmid, []).append(f1[1 + i])
            a0 = 1 + nmid
            run_pass(lhsA, asmA, emitA, mid, [f1[a0:a0 + 4], f1[a0 + 4:a0 + 8]])
            outA = [_mm(_unpack(OA[...]), _unpack(wo[j])) for j in range(KT)]
            memB = jnp.concatenate([a[0:8] for a in outA], axis=1)
            for f in f1[a0 + 8:]:
                f()

            lhsB = jnp.concatenate([memB, xnB], axis=0).astype(BF)

            def asmB(r, idx):
                return jnp.concatenate([r[0:8], carry[:, idx * 128:(idx + 1) * 128], r[8:32]], axis=0)

            def emitB(h, o):
                OB[:, h * 128:(h + 1) * 128] = _pack(jnp.concatenate(
                    [o[0:8], oleft[:, h * 128:(h + 1) * 128], o[8:40]], axis=0))

            f2 = [functools.partial(ffn2, j) for j in range(KT)]
            run_pass(lhsB, asmB, emitB, {}, [f2[0:1], f2[1:2]])
            for j in range(KT):
                cols = slice(j * 128, (j + 1) * 128)
                ob = _mm(_unpack(OB[...]), _unpack(wo[j]))
                if j + 2 < KT:
                    f2[j + 2]()
                mem_s[:, cols] = ob[0:8]
                att = jnp.concatenate([ob[8:16], outA[j][8:32], ob[16:48]], axis=0)
                ff = jnp.concatenate([FFO[_ds(it * 32, 32, 32), cols], FF[:, cols]], axis=0)
                xr = XR[it, :, cols].astype(F32)
                XR[it, :, cols] = (xr + att + ff).astype(BF)

        def loop_body(it, _):
            main_body(it)
            pltpu.make_async_copy(XR.at[it], o_h.at[it], sems.at[S_OUT]).start()
            return 0
        lax.fori_loop(0, NB, loop_body, 0)
        pltpu.make_async_copy(XR, o_h, sems.at[S_OUT]).wait()

    scratch = [
        pltpu.VMEM((3 * H, Dm // 2, 128), U32),
        pltpu.VMEM((KT, HD, 128), BF),
        pltpu.VMEM((FT, Dm, 128), BF),
        pltpu.VMEM((KT, F, 128), BF),
        pltpu.VMEM((3 * Dm * H, Dh), BF),
        pltpu.VMEM((NB, 64, Dm), BF),
        pltpu.VMEM((S, Dm), F32),
        pltpu.VMEM((S // 8, Dm), U32),
        pltpu.VMEM((S // 8, Dm), U32),
        pltpu.VMEM((S // 4, Dm), U32),
        pltpu.VMEM((4, 128, F), U32),
        pltpu.VMEM((S // 2, Dm), F32),
        pltpu.SemaphoreType.DMA((NSEM,)),
        pltpu.VMEM((M, Dm), F32),
        pltpu.VMEM((8, 3 * HD), F32),
        pltpu.VMEM((8, HD), F32),
        pltpu.VMEM((16, HD), U32),
        pltpu.VMEM((24, HD), U32),
        pltpu.VMEM((16, F), U32),
        pltpu.VMEM((32, Dm), F32),
        pltpu.VMEM((FT, 128), F32),
        pltpu.VMEM((KT, 128), F32),
        pltpu.VMEM((8 * TR + 16, 128), U32),
        pltpu.VMEM((M, Dm), BF),
        pltpu.VMEM((FT, 128), BF),
        pltpu.VMEM((KT, 128), BF),
        pltpu.VMEM((8, 128), U32),
    ]
    return kernel, scratch


@functools.partial(jax.jit, static_argnames=("A_seg_len",))
def pallas_parallel_sum__memory_aug_recurrent_mem_tr__dense_activation_gelu__prompt_kernel(
    A_x, A_mem0, A_Wq, A_Wk, A_Wv, A_Wo, A_seg_len, B_x, B_w1, B_b1, B_w2, B_b2,
):
    del B_x
    Bn, S, Dm = A_x.shape
    _, H, Dh = A_Wq.shape
    M = A_mem0.shape[1]
    F = B_w1.shape[1]
    assert (Bn, S, Dm, H, Dh, M, A_seg_len, F) == (1, 2048, 1024, 32, 128, 8, 32, 3584)
    kernel, scratch = _make_kernel(S, Dm, H, Dh, M, A_seg_len, F)
    any_spec = pl.BlockSpec(memory_space=pl.ANY)
    out = pl.pallas_call(
        kernel,
        grid=(1,),
        in_specs=[any_spec] * 10,
        out_specs=any_spec,
        out_shape=jax.ShapeDtypeStruct((S // 64, 64, Dm), A_x.dtype),
        scratch_shapes=scratch,
        compiler_params=pltpu.CompilerParams(
            dimension_semantics=("arbitrary",),
            vmem_limit_bytes=120 * 1024 * 1024),
    )(A_mem0.reshape(M, Dm), B_b1.reshape(F // 128, 128), B_b2.reshape(Dm // 128, 128),
      A_x.reshape(S // 64, 64, Dm),
      A_Wq.reshape(Dm * H, Dh), A_Wk.reshape(Dm * H, Dh), A_Wv.reshape(Dm * H, Dh),
      A_Wo.reshape(H * Dh, Dm), B_w1, B_w2)
    return out.reshape(Bn, S, Dm)
```

```python
import functools

import jax
import jax.numpy as jnp
import numpy as np
from jax import lax
from jax.experimental import pallas as pl
from jax.experimental.pallas import tpu as pltpu

BF = jnp.bfloat16
F32 = jnp.float32
U32 = jnp.uint32
LOG2E = 1.4426950408889634


def _unpack(x):
    return pltpu.bitcast(x, BF)


def _pack(x):
    return pltpu.bitcast(x.astype(BF), U32)


def _mm(a, b):
    return jnp.dot(a, b, preferred_element_type=F32)


def _gelu(x):
    c = 0.7978845608028654
    return 0.5 * x * (1.0 + jnp.tanh(c * (x + 0.044715 * (x * x * x))))


def _ds(start, size, mult):
    if isinstance(start, int):
        return pl.ds(start, size)
    return pl.ds(pl.multiple_of(start, mult), size)


def _spread(nslots, thunks):
    out = [[] for _ in range(nslots)]
    for i, f in enumerate(thunks):
        out[(i * nslots) // len(thunks)].append(f)
    return out


def _make_kernel(S, Dm, H, Dh, M, seg, F):
    KT = Dm // 128
    FT = F // 128
    HD = H * Dh
    L = M + seg
    NB = S // (2 * seg)
    NP = H // 2
    TR = 72
    c_soft = float(Dh) ** -0.5 * LOG2E
    PG, G2, GL = (1, 2, 5), 8, 5

    S_X, S_SM, S_W1 = 0, 6, 9
    S_W2 = S_W1 + FT
    S_QKV = S_W2 + KT
    S_WO = S_QKV + 48
    S_OUT = S_WO + KT
    NSEM = S_OUT + 1

    def kernel(mem0_h, b1_h, b2_h, x_h, wq_h, wk_h, wv_h, wo_h, w1_h, w2_h,
               o_h,
               wqkv, wo_b, w1_b, w2_b, stg, XR, XN, XBlo0, XBlo1, XBhi, Hp, FFO, sems,
               mem_s, carry, oleft, OA, OB, Hs, FF, B1f, B2f, RT,
               mem0_v, b1_v, b2_v, ZM):
        wo, w1, w2 = wo_b.bitcast(U32), w1_b.bitcast(U32), w2_b.bitcast(U32)

        def wait_like(ref, sem):
            pltpu.make_async_copy(ref, ref, sem).wait()

        def layernorm16(blk, part):
            x = XR[blk, _ds(part * 16, 16, 16), :].astype(F32)
            mu = jnp.mean(x, axis=-1, keepdims=True)
            xc = x - mu
            var = jnp.mean(xc * xc, axis=-1, keepdims=True)
            xn = xc * lax.rsqrt(var + 1e-5)
            XN[_ds(blk * 64 + part * 16, 16, 16), :] = xn
            return xn

        def token(xn):
            bits = pltpu.bitcast(xn, U32)
            acc = None
            for rr in range(xn.shape[0] // 8):
                for cc in range(KT):
                    v_ = bits[rr * 8:(rr + 1) * 8, cc * 128:(cc + 1) * 128]
                    acc = v_ if acc is None else (acc | v_)
            return acc

        def ln_lo(dst, blk, blk0, part):
            xn = layernorm16(blk, part)
            dst[_ds((blk - blk0) * 16 + 8 * part, 8, 8), :] = _pack(xn)
            return xn

        def ln_side_lo(blk, part):
            return token(ln_lo(XBlo1, blk, 16, part))

        def ln_side_hi(blk, part):
            xn = layernorm16(blk, 2 + part)
            XBhi[_ds(blk * 16 + 8 * part, 8, 8), :] = _pack(xn)
            return token(xn)

        def retile_store(p, buf):
            blk = stg.bitcast(U32).at[_ds(p * 256, 256, 256)]
            for u in range(2):
                for pp in range(8):
                    A = blk[pl.ds((2 * pp) * 16 + 8 * u, 8), :]
                    B = blk[pl.ds((2 * pp + 1) * 16 + 8 * u, 8), :]
                    lo = (A & 0xFFFF) | (B << 16)
                    hi = (A >> 16) | (B & np.uint32(0xFFFF0000))
                    RT[pl.ds((buf * 4 + u * 2) * TR + 9 * pp, 8), :] = lo
                    RT[pl.ds((buf * 4 + u * 2 + 1) * TR + 9 * pp, 8), :] = hi

        def retile_load(p, buf):
            m = p // 64
            r0 = (p % 64) * 8
            for u in range(2):
                for i in range(8):
                    for par in range(2):
                        v = RT[pl.ds((buf * 4 + u * 2 + par) * TR + i, 8, stride=9), :]
                        wqkv[m * H + 2 * (8 * u + i) + par, _ds(r0, 8, 8), :] = v

        cxlo = [pltpu.make_async_copy(x_h.at[4 * i:4 * i + 4, 0:32], XR.at[4 * i:4 * i + 4, 0:32],
                                      sems.at[S_X + i]) for i in range(4)]
        cx1lo = pltpu.make_async_copy(x_h.at[16:32, 0:32], XR.at[16:32, 0:32], sems.at[S_X + 4])
        cxhi = pltpu.make_async_copy(x_h.at[:, 32:64], XR.at[:, 32:64], sems.at[S_X + 5])
        csm = [pltpu.make_async_copy(h_, v_, sems.at[S_SM + i])
               for i, (h_, v_) in enumerate(((mem0_h, mem0_v), (b1_h, b1_v), (b2_h, b2_v)))]
        cw1 = [pltpu.make_async_copy(w1_h.at[:, pl.ds(j * 128, 128)], w1_b.at[j], sems.at[S_W1 + j])
               for j in range(FT)]
        cw2 = [pltpu.make_async_copy(w2_h.at[:, pl.ds(j * 128, 128)], w2_b.at[j], sems.at[S_W2 + j])
               for j in range(KT)]
        cq = [[pltpu.make_async_copy(wh.at[pl.ds(c * 2048, 2048)],
                                     stg.at[pl.ds((m * 16 + c) * 2048, 2048)],
                                     sems.at[S_QKV + m * 16 + c]) for c in range(16)]
              for m, wh in enumerate((wq_h, wk_h, wv_h))]
        cwo = [pltpu.make_async_copy(wo_h.at[:, pl.ds(j * 128, 128)], wo_b.at[j], sems.at[S_WO + j])
               for j in range(KT)]

        for c in cxlo + cw1[0:PG[0]] + csm + cw1[PG[0]:G2 + GL]:
            c.start()
        cx1lo.start()
        for c in cw1[G2 + GL:]:
            c.start()
        cxhi.start()

        def ln0_body(i, _):
            wait_like(XR.at[0:4, 0:32], sems.at[S_X + i])
            for bb in range(4):
                for part in range(2):
                    ln_lo(XBlo0, 4 * i + bb, 0, part)
            return 0
        lax.fori_loop(0, 4, ln0_body, 0)
        for c in csm:
            c.wait()
        ZM[...] = jnp.zeros((8, 128), U32)
        mem_s[...] = mem0_v[...].astype(F32)
        B1f[...] = b1_v[...].astype(F32)
        B2f[...] = b2_v[...].astype(F32)
        for c in cq[0]:
            c.start()
        for c in cw2:
            c.start()

        def ffn1_group(b, j0, nt, side):
            src = (XBlo0, XBlo1)[b]
            sl = (_spread(2 * nt - 1, side) + [[]]) if side else [[]] * (2 * nt)
            toks = {}
            for half in range(2):
                lhs = _unpack(src[pl.ds(half * 128, 128), :])
                for t in range(nt):
                    j = j0 + t
                    si = half * nt + t
                    bias = B1f[pl.ds(j, 1), :]
                    if toks.get(si - 1):
                        z = None
                        for tk in toks[si - 1]:
                            z = tk if z is None else (z | tk)
                        bias = bias + pltpu.bitcast(z & ZM[...], F32)[0:1, :]
                    hh = _mm(lhs, _unpack(w1[j])) + bias
                    toks[si] = [r for r in (f() for f in sl[si]) if r is not None]
                    Hp[b * 2 + half, :, _ds(j * 128, 128, 128)] = _pack(_gelu(hh))

        def ffn2_group(b, g, side):
            sl = _spread(4, side)
            for half in range(2):
                for t in range(2):
                    n = g * 2 + t
                    ff = _mm(_unpack(Hp[b * 2 + half]), _unpack(w2[n]))
                    for f in sl[half * 2 + t]:
                        f()
                    FFO[_ds(b * 512 + half * 256, 256, 256), _ds(n * 128, 128, 128)] = ff + B2f[pl.ds(n, 1), :]

        def retile_side(p0):
            for t in range(6):
                wait_like(stg.at[pl.ds(0, 2048)], sems.at[S_QKV + p0 // 4 + t])

            def step(t):
                def f():
                    if t < 24:
                        retile_store(p0 + t, t % 2)
                    if t >= 1:
                        retile_load(p0 + t - 1, (t - 1) % 2)
                return f
            return [step(t) for t in range(25)]

        j0 = 0
        for nt in PG:
            for c in cw1[j0:j0 + nt]:
                c.wait()
            ffn1_group(0, j0, nt, [])
            j0 += nt
        cx1lo.wait()

        def p10_body(i, _):
            for t in range(GL):
                wait_like(w1_b.at[0], sems.at[S_W1 + G2 + i * GL + t])
            ffn1_group(0, G2 + i * GL, GL,
                       [functools.partial(ln_side_lo, 16 + 4 * i + k // 2, k % 2) for k in range(8)])
            return 0
        lax.fori_loop(0, 4, p10_body, 0)

        for c in cq[1] + cq[2] + cwo:
            c.start()
        cxhi.wait()

        def p11_body(g, _):
            ffn1_group(1, g * (FT // 2), FT // 2,
                       [functools.partial(ln_side_hi, 16 * g + k // 2, k % 2) for k in range(32)])
            return 0
        lax.fori_loop(0, 2, p11_body, 0)
        for c in cw2:
            c.wait()

        def p2_body(i, _):
            ffn2_group(i // 4, i % 4, retile_side(i * 24))
            return 0
        lax.fori_loop(0, 8, p2_body, 0)
        for c in cwo:
            c.wait()

        def main_body(it):
            r64 = it * 64
            xnA = XN[_ds(r64, 40, 64), :]
            xnB = XN[_ds(r64 + 40, 24, 8), :]
            xh = _unpack(XBhi[_ds(it * 16, 16, 16), :])

            row = lax.broadcasted_iota(jnp.int32, (2 * L, 2 * L), 0)
            col = lax.broadcasted_iota(jnp.int32, (2 * L, 2 * L), 1)
            rowh = jnp.where(row >= L, row - L, row)
            colh = jnp.where(col >= L, col - L, col)
            same = (row >= L) == (col >= L)
            keep = ((rowh < M) | (rowh >= colh)) & same
            fill = jnp.where(same, -1e9 * LOG2E, -1e30)

            def softmax_parts(q, k):
                s = lax.dot_general(q, k, (((1,), (1,)), ((), ())), preferred_element_type=F32)
                s = jnp.where(keep, s * c_soft, fill)
                m = jnp.max(s, axis=-1, keepdims=True)
                e = jnp.exp2(s - m)
                l = jnp.sum(e, axis=-1, keepdims=True)
                r = pl.reciprocal(l, approx=True)
                r = r * (2.0 - l * r)
                return e.astype(BF), r

            def ffn1(j):
                hh = _mm(xh, _unpack(w1[j])) + B1f[j:j + 1, :]
                Hs[:, j * 128:(j + 1) * 128] = _pack(_gelu(hh))

            def ffn2(j):
                FF[:, j * 128:(j + 1) * 128] = _mm(_unpack(Hs[...]), _unpack(w2[j])) + B2f[j:j + 1, :]

            def run_pass(lhs, asm, emit, mid, fill_work):
                st = {}

                def proj2(base, t):
                    r0 = asm(_mm(lhs, _unpack(wqkv[base + 2 * t])), base + 2 * t)
                    r1 = asm(_mm(lhs, _unpack(wqkv[base + 2 * t + 1])), base + 2 * t + 1)
                    return jnp.concatenate([r0, r1], axis=0).astype(BF)

                for t in range(NP + 2):
                    if t < NP:
                        q = proj2(0, t)
                    else:
                        for f in fill_work[t - NP]:
                            f()
                    if 1 <= t <= NP:
                        st[t - 1]['e'], st[t - 1]['r'] = softmax_parts(st[t - 1]['q'], st[t - 1]['k'])
                    if t < NP:
                        k = proj2(H, t)
                        v = proj2(2 * H, t)
                        st[t] = dict(q=q, k=k, v=v)
                        for f in mid.get(t, []):
                            f()
                    if 2 <= t <= NP + 1:
                        d = st.pop(t - 2)
                        o = _mm(d['e'], d['v']) * d['r']
                        emit(2 * (t - 2), o[0:L])
                        emit(2 * (t - 2) + 1, o[L:2 * L])

            f1 = [functools.partial(ffn1, j) for j in range(FT)]
            f1[0]()
            lhsA = jnp.concatenate([mem_s[...], xnA], axis=0).astype(BF)

            def asmA(r, idx):
                carry[:, idx * 128:(idx + 1) * 128] = r[L:L + 8]
                return r[0:L]

            def emitA(h, o):
                OA[:, h * 128:(h + 1) * 128] = _pack(jnp.concatenate([o[0:8], o[16:40]], axis=0))
                oleft[:, h * 128:(h + 1) * 128] = o[8:16]

            nmid = FT - 17
            mid = {}
            for i in range(nmid):
                mid.setdefault((i * NP) // nmid, []).append(f1[1 + i])
            a0 = 1 + nmid
            run_pass(lhsA, asmA, emitA, mid, [f1[a0:a0 + 4], f1[a0 + 4:a0 + 8]])
            outA = [_mm(_unpack(OA[...]), _unpack(wo[j])) for j in range(KT)]
            memB = jnp.concatenate([a[0:8] for a in outA], axis=1)
            for f in f1[a0 + 8:]:
                f()

            lhsB = jnp.concatenate([memB, xnB], axis=0).astype(BF)

            def asmB(r, idx):
                return jnp.concatenate([r[0:8], carry[:, idx * 128:(idx + 1) * 128], r[8:32]], axis=0)

            def emitB(h, o):
                OB[:, h * 128:(h + 1) * 128] = _pack(jnp.concatenate(
                    [o[0:8], oleft[:, h * 128:(h + 1) * 128], o[8:40]], axis=0))

            f2 = [functools.partial(ffn2, j) for j in range(KT)]
            run_pass(lhsB, asmB, emitB, {}, [f2[0:1], f2[1:2]])
            for j in range(KT):
                cols = slice(j * 128, (j + 1) * 128)
                ob = _mm(_unpack(OB[...]), _unpack(wo[j]))
                if j + 2 < KT:
                    f2[j + 2]()
                mem_s[:, cols] = ob[0:8]
                att = jnp.concatenate([ob[8:16], outA[j][8:32], ob[16:48]], axis=0)
                ff = jnp.concatenate([FFO[_ds(it * 32, 32, 32), cols], FF[:, cols]], axis=0)
                xr = XR[it, :, cols].astype(F32)
                XR[it, :, cols] = (xr + att + ff).astype(BF)

        def loop_body(it, _):
            main_body(it)
            pltpu.make_async_copy(XR.at[it], o_h.at[it], sems.at[S_OUT]).start()
            return 0
        lax.fori_loop(0, NB, loop_body, 0)
        pltpu.make_async_copy(XR, o_h, sems.at[S_OUT]).wait()

    scratch = [
        pltpu.VMEM((3 * H, Dm // 2, 128), U32),
        pltpu.VMEM((KT, HD, 128), BF),
        pltpu.VMEM((FT, Dm, 128), BF),
        pltpu.VMEM((KT, F, 128), BF),
        pltpu.VMEM((3 * Dm * H, Dh), BF),
        pltpu.VMEM((NB, 64, Dm), BF),
        pltpu.VMEM((S, Dm), F32),
        pltpu.VMEM((S // 8, Dm), U32),
        pltpu.VMEM((S // 8, Dm), U32),
        pltpu.VMEM((S // 4, Dm), U32),
        pltpu.VMEM((4, 128, F), U32),
        pltpu.VMEM((S // 2, Dm), F32),
        pltpu.SemaphoreType.DMA((NSEM,)),
        pltpu.VMEM((M, Dm), F32),
        pltpu.VMEM((8, 3 * HD), F32),
        pltpu.VMEM((8, HD), F32),
        pltpu.VMEM((16, HD), U32),
        pltpu.VMEM((24, HD), U32),
        pltpu.VMEM((16, F), U32),
        pltpu.VMEM((32, Dm), F32),
        pltpu.VMEM((FT, 128), F32),
        pltpu.VMEM((KT, 128), F32),
        pltpu.VMEM((8 * TR + 16, 128), U32),
        pltpu.VMEM((M, Dm), BF),
        pltpu.VMEM((FT, 128), BF),
        pltpu.VMEM((KT, 128), BF),
        pltpu.VMEM((8, 128), U32),
    ]
    return kernel, scratch


@functools.partial(jax.jit, static_argnames=("A_seg_len",))
def pallas_parallel_sum__memory_aug_recurrent_mem_tr__dense_activation_gelu__prompt_kernel(
    A_x, A_mem0, A_Wq, A_Wk, A_Wv, A_Wo, A_seg_len, B_x, B_w1, B_b1, B_w2, B_b2,
):
    del B_x
    Bn, S, Dm = A_x.shape
    _, H, Dh = A_Wq.shape
    M = A_mem0.shape[1]
    F = B_w1.shape[1]
    assert (Bn, S, Dm, H, Dh, M, A_seg_len, F) == (1, 2048, 1024, 32, 128, 8, 32, 3584)
    kernel, scratch = _make_kernel(S, Dm, H, Dh, M, A_seg_len, F)
    any_spec = pl.BlockSpec(memory_space=pl.ANY)
    out = pl.pallas_call(
        kernel,
        grid=(1,),
        in_specs=[any_spec] * 10,
        out_specs=any_spec,
        out_shape=jax.ShapeDtypeStruct((S // 64, 64, Dm), A_x.dtype),
        scratch_shapes=scratch,
        compiler_params=pltpu.CompilerParams(
            dimension_semantics=("arbitrary",),
            vmem_limit_bytes=120 * 1024 * 1024),
    )(A_mem0.reshape(M, Dm), B_b1.reshape(F // 128, 128), B_b2.reshape(Dm // 128, 128),
      A_x.reshape(S // 64, 64, Dm),
      A_Wq.reshape(Dm * H, Dh), A_Wk.reshape(Dm * H, Dh), A_Wv.reshape(Dm * H, Dh),
      A_Wo.reshape(H * Dh, Dm), B_w1, B_w2)
    return out.reshape(Bn, S, Dm)
```

```python
import functools

import jax
import jax.numpy as jnp
import numpy as np
from jax import lax
from jax.experimental import pallas as pl
from jax.experimental.pallas import tpu as pltpu

BF = jnp.bfloat16
F32 = jnp.float32
U32 = jnp.uint32
LOG2E = 1.4426950408889634


def _unpack(x):
    return pltpu.bitcast(x, BF)


def _pack(x):
    return pltpu.bitcast(x.astype(BF), U32)


def _mm(a, b):
    return jnp.dot(a, b, preferred_element_type=F32)


def _gelu(x):
    c = 0.7978845608028654
    return 0.5 * x * (1.0 + jnp.tanh(c * (x + 0.044715 * (x * x * x))))


def _ds(start, size, mult):
    if isinstance(start, int):
        return pl.ds(start, size)
    return pl.ds(pl.multiple_of(start, mult), size)


def _spread(nslots, thunks):
    out = [[] for _ in range(nslots)]
    for i, f in enumerate(thunks):
        out[(i * nslots) // len(thunks)].append(f)
    return out


def _make_kernel(S, Dm, H, Dh, M, seg, F):
    KT = Dm // 128
    FT = F // 128
    HD = H * Dh
    L = M + seg
    NB = S // (2 * seg)
    NP = H // 2
    TR = 72
    c_soft = float(Dh) ** -0.5 * LOG2E
    PG, G2, GL = (1, 2, 5), 8, 5

    S_X, S_SM, S_W1 = 0, 6, 9
    S_W2 = S_W1 + FT
    S_QKV = S_W2 + KT
    S_WO = S_QKV + 48
    S_OUT = S_WO + KT
    NSEM = S_OUT + 1

    def kernel(mem0_h, b1_h, b2_h, x_h, wq_h, wk_h, wv_h, wo_h, w1_h, w2_h,
               o_h,
               wqkv, wo_b, w1_b, w2_b, stg, XR, XN, XBlo0, XBlo1, XBhi, Hp, FFO, sems,
               mem_s, carry, oleft, OA, OB, Hs, FF, B1f, B2f, RT,
               mem0_v, b1_v, b2_v, ZM):
        wo, w1, w2 = wo_b.bitcast(U32), w1_b.bitcast(U32), w2_b.bitcast(U32)

        def wait_into(dst, sem):
            pltpu.make_async_copy(dst, dst, sem).wait()

        def layernorm16(blk, part):
            x = XR[blk, _ds(part * 16, 16, 16), :].astype(F32)
            mu = jnp.mean(x, axis=-1, keepdims=True)
            xc = x - mu
            var = jnp.mean(xc * xc, axis=-1, keepdims=True)
            xn = xc * lax.rsqrt(var + 1e-5)
            XN[_ds(blk * 64 + part * 16, 16, 16), :] = xn
            return xn

        def token(xn):
            bits = pltpu.bitcast(xn, U32)
            acc = None
            for rr in range(xn.shape[0] // 8):
                for cc in range(KT):
                    v_ = bits[rr * 8:(rr + 1) * 8, cc * 128:(cc + 1) * 128]
                    acc = v_ if acc is None else (acc | v_)
            return acc

        def ln_lo(dst, blk, blk0, part):
            xn = layernorm16(blk, part)
            dst[_ds((blk - blk0) * 16 + 8 * part, 8, 8), :] = _pack(xn)
            return xn

        def ln_side_lo(blk, part):
            return token(ln_lo(XBlo1, blk, 16, part))

        def ln_side_hi(blk, part):
            xn = layernorm16(blk, 2 + part)
            XBhi[_ds(blk * 16 + 8 * part, 8, 8), :] = _pack(xn)
            return token(xn)

        def retile_store(p, buf):
            blk = stg.bitcast(U32).at[_ds(p * 256, 256, 256)]
            for u in range(2):
                for pp in range(8):
                    A = blk[pl.ds((2 * pp) * 16 + 8 * u, 8), :]
                    B = blk[pl.ds((2 * pp + 1) * 16 + 8 * u, 8), :]
                    lo = (A & 0xFFFF) | (B << 16)
                    hi = (A >> 16) | (B & np.uint32(0xFFFF0000))
                    RT[pl.ds((buf * 4 + u * 2) * TR + 9 * pp, 8), :] = lo
                    RT[pl.ds((buf * 4 + u * 2 + 1) * TR + 9 * pp, 8), :] = hi

        def retile_load(p, buf):
            m = p // 64
            r0 = (p % 64) * 8
            for u in range(2):
                for i in range(8):
                    for par in range(2):
                        v = RT[pl.ds((buf * 4 + u * 2 + par) * TR + i, 8, stride=9), :]
                        wqkv[m * H + 2 * (8 * u + i) + par, _ds(r0, 8, 8), :] = v

        cxlo = [pltpu.make_async_copy(x_h.at[4 * i:4 * i + 4, 0:32], XR.at[4 * i:4 * i + 4, 0:32],
                                      sems.at[S_X + i]) for i in range(4)]
        cx1lo = pltpu.make_async_copy(x_h.at[16:32, 0:32], XR.at[16:32, 0:32], sems.at[S_X + 4])
        cxhi = pltpu.make_async_copy(x_h.at[:, 32:64], XR.at[:, 32:64], sems.at[S_X + 5])
        csm = [pltpu.make_async_copy(h_, v_, sems.at[S_SM + i])
               for i, (h_, v_) in enumerate(((mem0_h, mem0_v), (b1_h, b1_v), (b2_h, b2_v)))]
        cw1 = [pltpu.make_async_copy(w1_h.at[:, pl.ds(j * 128, 128)], w1_b.at[j], sems.at[S_W1 + j])
               for j in range(FT)]
        cw2 = [pltpu.make_async_copy(w2_h.at[:, pl.ds(j * 128, 128)], w2_b.at[j], sems.at[S_W2 + j])
               for j in range(KT)]
        cq = [[pltpu.make_async_copy(wh.at[pl.ds(c * 2048, 2048)],
                                     stg.at[pl.ds((m * 16 + c) * 2048, 2048)],
                                     sems.at[S_QKV + m * 16 + c]) for c in range(16)]
              for m, wh in enumerate((wq_h, wk_h, wv_h))]
        cwo = [pltpu.make_async_copy(wo_h.at[:, pl.ds(j * 128, 128)], wo_b.at[j], sems.at[S_WO + j])
               for j in range(KT)]

        for c in cxlo + cw1[0:PG[0]] + csm + cw1[PG[0]:G2 + GL]:
            c.start()
        cx1lo.start()
        for c in cw1[G2 + GL:]:
            c.start()
        cxhi.start()

        def ln0_body(i, _):
            wait_into(XR.at[_ds(4 * i, 4, 4), 0:32], sems.at[S_X + i])
            for bb in range(4):
                for part in range(2):
                    ln_lo(XBlo0, 4 * i + bb, 0, part)
            return 0
        lax.fori_loop(0, 4, ln0_body, 0)
        for c in csm:
            c.wait()
        ZM[...] = jnp.zeros((8, 128), U32)
        mem_s[...] = mem0_v[...].astype(F32)
        B1f[...] = b1_v[...].astype(F32)
        B2f[...] = b2_v[...].astype(F32)
        for c in cq[0]:
            c.start()
        for c in cw2:
            c.start()

        def ffn1_group(b, j0, nt, side):
            src = (XBlo0, XBlo1)[b]
            sl = (_spread(2 * nt - 1, side) + [[]]) if side else [[]] * (2 * nt)
            toks = {}
            for half in range(2):
                lhs = _unpack(src[pl.ds(half * 128, 128), :])
                for t in range(nt):
                    j = j0 + t
                    si = half * nt + t
                    bias = B1f[pl.ds(j, 1), :]
                    if toks.get(si - 1):
                        z = None
                        for tk in toks[si - 1]:
                            z = tk if z is None else (z | tk)
                        bias = bias + pltpu.bitcast(z & ZM[...], F32)[0:1, :]
                    hh = _mm(lhs, _unpack(w1[j])) + bias
                    toks[si] = [r for r in (f() for f in sl[si]) if r is not None]
                    Hp[b * 2 + half, :, _ds(j * 128, 128, 128)] = _pack(_gelu(hh))

        def ffn2_group(b, g, side):
            sl = _spread(4, side)
            for half in range(2):
                for t in range(2):
                    n = g * 2 + t
                    ff = _mm(_unpack(Hp[b * 2 + half]), _unpack(w2[n]))
                    for f in sl[half * 2 + t]:
                        f()
                    FFO[_ds(b * 512 + half * 256, 256, 256), _ds(n * 128, 128, 128)] = ff + B2f[pl.ds(n, 1), :]

        def retile_side(p0):
            for t in range(6):
                wait_into(stg.at[_ds((p0 // 4 + t) * 2048, 2048, 2048)], sems.at[S_QKV + p0 // 4 + t])

            def step(t):
                def f():
                    if t < 24:
                        retile_store(p0 + t, t % 2)
                    if t >= 1:
                        retile_load(p0 + t - 1, (t - 1) % 2)
                return f
            return [step(t) for t in range(25)]

        j0 = 0
        for nt in PG:
            for c in cw1[j0:j0 + nt]:
                c.wait()
            ffn1_group(0, j0, nt, [])
            j0 += nt
        cx1lo.wait()

        def p10_body(i, _):
            for t in range(GL):
                wait_into(w1_b.at[G2 + i * GL + t], sems.at[S_W1 + G2 + i * GL + t])
            ffn1_group(0, G2 + i * GL, GL,
                       [functools.partial(ln_side_lo, 16 + 4 * i + k // 2, k % 2) for k in range(8)])
            return 0
        lax.fori_loop(0, 4, p10_body, 0)

        for c in cq[1] + cq[2] + cwo:
            c.start()
        cxhi.wait()

        def p11_body(g, _):
            ffn1_group(1, g * (FT // 2), FT // 2,
                       [functools.partial(ln_side_hi, 16 * g + k // 2, k % 2) for k in range(32)])
            return 0
        lax.fori_loop(0, 2, p11_body, 0)
        for c in cw2:
            c.wait()

        def p2_body(i, _):
            ffn2_group(i // 4, i % 4, retile_side(i * 24))
            return 0
        lax.fori_loop(0, 8, p2_body, 0)
        for c in cwo:
            c.wait()

        def main_body(it):
            r64 = it * 64
            xnA = XN[_ds(r64, 40, 64), :]
            xnB = XN[_ds(r64 + 40, 24, 8), :]
            xh = _unpack(XBhi[_ds(it * 16, 16, 16), :])

            row = lax.broadcasted_iota(jnp.int32, (2 * L, 2 * L), 0)
            col = lax.broadcasted_iota(jnp.int32, (2 * L, 2 * L), 1)
            rowh = jnp.where(row >= L, row - L, row)
            colh = jnp.where(col >= L, col - L, col)
            same = (row >= L) == (col >= L)
            keep = ((rowh < M) | (rowh >= colh)) & same
            fill = jnp.where(same, -1e9 * LOG2E, -1e30)

            def softmax_parts(q, k):
                s = lax.dot_general(q, k, (((1,), (1,)), ((), ())), preferred_element_type=F32)
                s = jnp.where(keep, s * c_soft, fill)
                m = jnp.max(s, axis=-1, keepdims=True)
                e = jnp.exp2(s - m)
                l = jnp.sum(e, axis=-1, keepdims=True)
                r = pl.reciprocal(l, approx=True)
                r = r * (2.0 - l * r)
                return e.astype(BF), r

            def ffn1(j):
                hh = _mm(xh, _unpack(w1[j])) + B1f[j:j + 1, :]
                Hs[:, j * 128:(j + 1) * 128] = _pack(_gelu(hh))

            def ffn2(j):
                FF[:, j * 128:(j + 1) * 128] = _mm(_unpack(Hs[...]), _unpack(w2[j])) + B2f[j:j + 1, :]

            def run_pass(lhs, asm, emit, mid, fill_work):
                st = {}

                def proj2(base, t):
                    r0 = asm(_mm(lhs, _unpack(wqkv[base + 2 * t])), base + 2 * t)
                    r1 = asm(_mm(lhs, _unpack(wqkv[base + 2 * t + 1])), base + 2 * t + 1)
                    return jnp.concatenate([r0, r1], axis=0).astype(BF)

                for t in range(NP + 2):
                    if t < NP:
                        q = proj2(0, t)
                    else:
                        for f in fill_work[t - NP]:
                            f()
                    if 1 <= t <= NP:
                        st[t - 1]['e'], st[t - 1]['r'] = softmax_parts(st[t - 1]['q'], st[t - 1]['k'])
                    if t < NP:
                        k = proj2(H, t)
                        v = proj2(2 * H, t)
                        st[t] = dict(q=q, k=k, v=v)
                        for f in mid.get(t, []):
                            f()
                    if 2 <= t <= NP + 1:
                        d = st.pop(t - 2)
                        o = _mm(d['e'], d['v']) * d['r']
                        emit(2 * (t - 2), o[0:L])
                        emit(2 * (t - 2) + 1, o[L:2 * L])

            f1 = [functools.partial(ffn1, j) for j in range(FT)]
            f1[0]()
            lhsA = jnp.concatenate([mem_s[...], xnA], axis=0).astype(BF)

            def asmA(r, idx):
                carry[:, idx * 128:(idx + 1) * 128] = r[L:L + 8]
                return r[0:L]

            def emitA(h, o):
                OA[:, h * 128:(h + 1) * 128] = _pack(jnp.concatenate([o[0:8], o[16:40]], axis=0))
                oleft[:, h * 128:(h + 1) * 128] = o[8:16]

            nmid = FT - 17
            mid = {}
            for i in range(nmid):
                mid.setdefault((i * NP) // nmid, []).append(f1[1 + i])
            a0 = 1 + nmid
            run_pass(lhsA, asmA, emitA, mid, [f1[a0:a0 + 4], f1[a0 + 4:a0 + 8]])
            outA = [_mm(_unpack(OA[...]), _unpack(wo[j])) for j in range(KT)]
            memB = jnp.concatenate([a[0:8] for a in outA], axis=1)
            for f in f1[a0 + 8:]:
                f()

            lhsB = jnp.concatenate([memB, xnB], axis=0).astype(BF)

            def asmB(r, idx):
                return jnp.concatenate([r[0:8], carry[:, idx * 128:(idx + 1) * 128], r[8:32]], axis=0)

            def emitB(h, o):
                OB[:, h * 128:(h + 1) * 128] = _pack(jnp.concatenate(
                    [o[0:8], oleft[:, h * 128:(h + 1) * 128], o[8:40]], axis=0))

            f2 = [functools.partial(ffn2, j) for j in range(KT)]
            run_pass(lhsB, asmB, emitB, {}, [f2[0:1], f2[1:2]])
            for j in range(KT):
                cols = slice(j * 128, (j + 1) * 128)
                ob = _mm(_unpack(OB[...]), _unpack(wo[j]))
                if j + 2 < KT:
                    f2[j + 2]()
                mem_s[:, cols] = ob[0:8]
                att = jnp.concatenate([ob[8:16], outA[j][8:32], ob[16:48]], axis=0)
                ff = jnp.concatenate([FFO[_ds(it * 32, 32, 32), cols], FF[:, cols]], axis=0)
                xr = XR[it, :, cols].astype(F32)
                XR[it, :, cols] = (xr + att + ff).astype(BF)

        def loop_body(it, _):
            main_body(it)
            pltpu.make_async_copy(XR.at[it], o_h.at[it], sems.at[S_OUT]).start()
            return 0
        lax.fori_loop(0, NB, loop_body, 0)
        pltpu.make_async_copy(XR, o_h, sems.at[S_OUT]).wait()

    scratch = [
        pltpu.VMEM((3 * H, Dm // 2, 128), U32),
        pltpu.VMEM((KT, HD, 128), BF),
        pltpu.VMEM((FT, Dm, 128), BF),
        pltpu.VMEM((KT, F, 128), BF),
        pltpu.VMEM((3 * Dm * H, Dh), BF),
        pltpu.VMEM((NB, 64, Dm), BF),
        pltpu.VMEM((S, Dm), F32),
        pltpu.VMEM((S // 8, Dm), U32),
        pltpu.VMEM((S // 8, Dm), U32),
        pltpu.VMEM((S // 4, Dm), U32),
        pltpu.VMEM((4, 128, F), U32),
        pltpu.VMEM((S // 2, Dm), F32),
        pltpu.SemaphoreType.DMA((NSEM,)),
        pltpu.VMEM((M, Dm), F32),
        pltpu.VMEM((8, 3 * HD), F32),
        pltpu.VMEM((8, HD), F32),
        pltpu.VMEM((16, HD), U32),
        pltpu.VMEM((24, HD), U32),
        pltpu.VMEM((16, F), U32),
        pltpu.VMEM((32, Dm), F32),
        pltpu.VMEM((FT, 128), F32),
        pltpu.VMEM((KT, 128), F32),
        pltpu.VMEM((8 * TR + 16, 128), U32),
        pltpu.VMEM((M, Dm), BF),
        pltpu.VMEM((FT, 128), BF),
        pltpu.VMEM((KT, 128), BF),
        pltpu.VMEM((8, 128), U32),
    ]
    return kernel, scratch


@functools.partial(jax.jit, static_argnames=("A_seg_len",))
def pallas_parallel_sum__memory_aug_recurrent_mem_tr__dense_activation_gelu__prompt_kernel(
    A_x, A_mem0, A_Wq, A_Wk, A_Wv, A_Wo, A_seg_len, B_x, B_w1, B_b1, B_w2, B_b2,
):
    del B_x
    Bn, S, Dm = A_x.shape
    _, H, Dh = A_Wq.shape
    M = A_mem0.shape[1]
    F = B_w1.shape[1]
    assert (Bn, S, Dm, H, Dh, M, A_seg_len, F) == (1, 2048, 1024, 32, 128, 8, 32, 3584)
    kernel, scratch = _make_kernel(S, Dm, H, Dh, M, A_seg_len, F)
    any_spec = pl.BlockSpec(memory_space=pl.ANY)
    out = pl.pallas_call(
        kernel,
        grid=(1,),
        in_specs=[any_spec] * 10,
        out_specs=any_spec,
        out_shape=jax.ShapeDtypeStruct((S // 64, 64, Dm), A_x.dtype),
        scratch_shapes=scratch,
        compiler_params=pltpu.CompilerParams(
            dimension_semantics=("arbitrary",),
            vmem_limit_bytes=120 * 1024 * 1024),
    )(A_mem0.reshape(M, Dm), B_b1.reshape(F // 128, 128), B_b2.reshape(Dm // 128, 128),
      A_x.reshape(S // 64, 64, Dm),
      A_Wq.reshape(Dm * H, Dh), A_Wk.reshape(Dm * H, Dh), A_Wv.reshape(Dm * H, Dh),
      A_Wo.reshape(H * Dh, Dm), B_w1, B_w2)
    return out.reshape(Bn, S, Dm)
```
